```python
import jax
import jax.numpy as jnp

def _softmax(x, axis=-1):
    return jax.nn.softmax(x, axis=axis)
def _gelu(x):
    return jax.nn.gelu(x, approximate=True)
def _silu(x):
    return jax.nn.silu(x)
def _sigmoid(x):
    return jax.nn.sigmoid(x)
def _layernorm(x, axis=-1, eps=1e-5):
    m = jnp.mean(x, axis=axis, keepdims=True)
    v = jnp.var(x, axis=axis, keepdims=True)
    return (x - m) / jnp.sqrt(v + eps)
def _scatter_add(tgt, idx, src, axis=0):
    return tgt.at[idx].add(src)
def _segment_sum(src, seg, n):
    return jax.ops.segment_sum(src, seg, n)
class _Rng:
    def __init__(self, key):
        self._k = key
    def _next(self):
        self._k, sub = jax.random.split(self._k)
        return sub
    def normal(self, shape):
        return jax.random.normal(self._next(), shape, dtype=jnp.bfloat16)
    def randint(self, lo, hi, shape):
        return jax.random.randint(self._next(), shape, lo, hi, dtype=jnp.int32)
    def uniform(self, shape, lo=0.0, hi=1.0):
        return jax.random.uniform(self._next(), shape, jnp.bfloat16, lo, hi)
    def permutation(self, n):
        return jax.random.permutation(self._next(), n)


kernel_name = 'sequential_preLN__sliding_block_cached__mixer_s_mlp__decode'

def setup_inputs():
    _rng = _Rng(jax.random.key(int.from_bytes(__import__("os").urandom(4), "little")))
    _w = (lambda a: (lambda t: t.astype(jnp.bfloat16) if jnp.issubdtype(t.dtype, jnp.floating) else t)(jnp.asarray(a)))
    def _A_setup():
        B, Sq, D = 1, 1, 640
        Hq, Hkv, Sk, Dh = 32, 32, 32768, 192
        assert Hq % Hkv == 0, (Hq, Hkv)
        return {
            "x": _w((lambda *s: _rng.normal(s) * 0.05)(B, Sq, D)),
            "k_cache": _w((lambda *s: _rng.normal(s) * 0.05)(B, Hkv, Sk, Dh)),
            "v_cache": _w((lambda *s: _rng.normal(s) * 0.05)(B, Hkv, Sk, Dh)),
            "wq": _w((lambda *s: _rng.normal(s) * 0.05)(D, Hq * Dh) * (D ** -0.5)),
            "wo": _w((lambda *s: _rng.normal(s) * 0.05)(Hq * Dh, D) * ((Hq * Dh) ** -0.5)),
        }
    _A_in = _A_setup()

    def _B_setup():
        B, S, D, F = 1, 1, 640, 1536
        return {
            "x":  _w((lambda *s: _rng.normal(s) * 0.05)(B, S, D)),
            "w1": _w((lambda *s: _rng.normal(s) * 0.05)(D, D) * (D ** -0.5)),
            "w2": _w((lambda *s: _rng.normal(s) * 0.05)(D, D) * (D ** -0.5)),
            "w3": _w((lambda *s: _rng.normal(s) * 0.05)(D, F) * (D ** -0.5)),
            "w4": _w((lambda *s: _rng.normal(s) * 0.05)(F, D) * (F ** -0.5)),
        }
    _B_in = _B_setup()

    return {
        "A_x": _A_in["x"],
        "A_k_cache": _A_in["k_cache"],
        "A_v_cache": _A_in["v_cache"],
        "A_wq": _A_in["wq"],
        "A_wo": _A_in["wo"],
        "B_x": _B_in["x"],
        "B_w1": _B_in["w1"],
        "B_w2": _B_in["w2"],
        "B_w3": _B_in["w3"],
        "B_w4": _B_in["w4"],
    }

def reference(A_x, A_k_cache, A_v_cache, A_wq, A_wo, B_x, B_w1, B_w2, B_w3, B_w4):
    def _A_ref(x, k_cache, v_cache, wq, wo):
        B, Sq, D = x.shape
        Hq, Dh = 32, 192
        Hkv, Sk = k_cache.shape[1], k_cache.shape[2]
        W = min(4096, max(256, Sk // 4))
        rep = Hq // Hkv
        q = (lambda x, *d: x.transpose(*d))((x @ wq).reshape(B, Sq, Hq, Dh), 0, 2, 1, 3)
        k = jnp.repeat(k_cache[:, :, Sk - W:, :], rep, axis=1)
        v = jnp.repeat(v_cache[:, :, Sk - W:, :], rep, axis=1)
        scores = jnp.einsum("bhqd,bhkd->bhqk", q, k) * (Dh ** -0.5)
        p = _softmax(scores, axis=-1)
        o = jnp.einsum("bhqk,bhkd->bhqd", p, v)
        return (lambda x, *d: x.transpose(*d))(o, 0, 2, 1, 3).reshape(B, Sq, Hq * Dh) @ wo

    def _B_ref(x, w1, w2, w3, w4):
        B, S, D = x.shape
        h = _gelu(_layernorm(x, axis=-1) @ w1)
        c = D // 4
        g0 = jnp.pad(h[:, :, 0*c:1*c], ((0, 0), (1, 0), (0, 0)))[:, :S, :]
        g1 = jnp.pad(h[:, :, 1*c:2*c], ((0, 0), (0, 1), (0, 0)))[:, 1:, :]
        g2 = jnp.pad(h[:, :, 2*c:3*c], ((0, 0), (2, 0), (0, 0)))[:, :S, :]
        g3 = jnp.pad(h[:, :, 3*c:   ], ((0, 0), (0, 2), (0, 0)))[:, 2:, :]
        hs = jnp.concatenate([g0, g1, g2, g3], axis=-1) @ w2
        x1 = x + hs
        h2 = _gelu(_layernorm(x1, axis=-1) @ w3) @ w4
        return x1 + h2

    x = A_x
    h = x + _A_ref(_layernorm(x, axis=-1), A_k_cache, A_v_cache, A_wq, A_wo)
    h2 = h + _B_ref(_layernorm(h, axis=-1), B_w1, B_w2, B_w3, B_w4)
    return h2
```

```python
import functools

import jax
import jax.numpy as jnp
from jax import lax
import jax.experimental.pallas as pl
import jax.experimental.pallas.tpu as pltpu

_F32 = jnp.float32
_BF16 = jnp.bfloat16
_EPS = 1e-5
_NB = 3
_ROWS = 8


def _layernorm(x):
    m = jnp.mean(x, axis=-1, keepdims=True)
    xc = x - m
    v = jnp.mean(xc * xc, axis=-1, keepdims=True)
    return xc / jnp.sqrt(v + _EPS)


def _w4_chunks(f):
    sizes = []
    rem = f
    for s in (512, 512, 256, 128):
        if rem > s:
            sizes.append(s)
            rem -= s
    sizes.append(rem)
    offs = [sum(sizes[:i]) for i in range(len(sizes))]
    return list(zip(offs, sizes))


def _kernel(x_hbm, kt_hbm, vt_hbm, wq_hbm, wo_hbm, w3_hbm, w4_hbm, o_ref,
            x_buf, wq_buf, wo_buf, w3_buf, w4_buf, k_buf, v_buf, q_scr,
            misc_sem, k_sem, v_sem, w4_sem, *, n_heads, dh, sk, win):
    start = sk - win
    scale = dh ** -0.5
    chunks = _w4_chunks(w4_buf.shape[0])

    x_cp = pltpu.make_async_copy(x_hbm, x_buf, misc_sem.at[0])
    wq_cp = pltpu.make_async_copy(wq_hbm, wq_buf, misc_sem.at[1])
    wo_cp = pltpu.make_async_copy(wo_hbm, wo_buf, misc_sem.at[2])
    w3_cp = pltpu.make_async_copy(w3_hbm, w3_buf, misc_sem.at[3])

    def w4_cp(i):
        off, size = chunks[i]
        return pltpu.make_async_copy(
            w4_hbm.at[pl.ds(off, size)], w4_buf.at[pl.ds(off, size)], w4_sem.at[i])

    def k_cp(h, slot):
        return pltpu.make_async_copy(
            kt_hbm.at[0, h, :, pl.ds(start, win)], k_buf.at[slot], k_sem.at[slot])

    def v_cp(h, slot):
        return pltpu.make_async_copy(
            vt_hbm.at[0, h, :, pl.ds(start, win)], v_buf.at[slot], v_sem.at[slot])

    x_cp.start()
    wq_cp.start()
    wo_cp.start()
    for h in range(_NB):
        k_cp(h, h).start()
        v_cp(h, h).start()

    x_cp.wait()
    x = jnp.broadcast_to(x_buf[0].astype(_F32), (_ROWS, x_buf.shape[-1]))
    xn = _layernorm(x).astype(_BF16)

    wq_cp.wait()
    q = jnp.dot(xn, wq_buf[...], preferred_element_type=_F32).astype(_BF16)
    for h in range(n_heads):
        q_scr[h] = q[:, h * dh:(h + 1) * dh]

    wo_cp.wait()

    def head(h, attn):
        slot = h % _NB
        k_cp(h, slot).wait()
        s = jnp.dot(q_scr[h], k_buf[slot], preferred_element_type=_F32) * scale

        @pl.when(h + _NB < n_heads)
        def _():
            k_cp(h + _NB, slot).start()

        m = jnp.max(s, axis=-1, keepdims=True)
        p = jnp.exp(s - m)
        l = jnp.sum(p, axis=-1, keepdims=True)

        v_cp(h, slot).wait()
        o = lax.dot_general(p.astype(_BF16), v_buf[slot], (((1,), (1,)), ((), ())),
                            preferred_element_type=_F32)

        @pl.when(h + _NB < n_heads)
        def _():
            v_cp(h + _NB, slot).start()

        @pl.when(h + _NB == n_heads - 1)
        def _():
            w3_cp.start()
            for i in range(len(chunks)):
                w4_cp(i).start()

        o = (o / l).astype(_BF16)
        row = pl.multiple_of(h * dh, 64)
        return attn + jnp.dot(o, wo_buf[pl.ds(row, dh), :], preferred_element_type=_F32)

    attn = lax.fori_loop(0, n_heads, head, jnp.zeros(x.shape, _F32))

    hres = x + attn
    y = _layernorm(hres)
    z = _layernorm(y).astype(_BF16)
    w3_cp.wait()
    g = jax.nn.gelu(jnp.dot(z, w3_buf[...], preferred_element_type=_F32),
                    approximate=True).astype(_BF16)
    out = hres + y
    for i, (off, size) in enumerate(chunks):
        w4_cp(i).wait()
        out = out + jnp.dot(g[:, off:off + size], w4_buf[off:off + size, :],
                            preferred_element_type=_F32)
    o_ref[0] = out[0:1].astype(o_ref.dtype)


@jax.jit
def pallas_sequential_preLN__sliding_block_cached__mixer_s_mlp__decode_kernel(
    A_x: jax.Array,
    A_k_cache: jax.Array,
    A_v_cache: jax.Array,
    A_wq: jax.Array,
    A_wo: jax.Array,
    B_x: jax.Array,
    B_w1: jax.Array,
    B_w2: jax.Array,
    B_w3: jax.Array,
    B_w4: jax.Array,
):
    b, sq, d = A_x.shape
    _, n_heads, sk, dh = A_k_cache.shape
    assert b == 1 and sq == 1 and A_wq.shape == (d, n_heads * dh)
    win = min(4096, max(256, sk // 4))
    f = B_w3.shape[1]

    kt = jnp.swapaxes(A_k_cache, 2, 3)
    vt = jnp.swapaxes(A_v_cache, 2, 3)

    any_spec = pl.BlockSpec(memory_space=pl.ANY)
    return pl.pallas_call(
        functools.partial(_kernel, n_heads=n_heads, dh=dh, sk=sk, win=win),
        in_specs=[any_spec] * 7,
        out_specs=pl.BlockSpec(memory_space=pltpu.VMEM),
        out_shape=jax.ShapeDtypeStruct(A_x.shape, A_x.dtype),
        scratch_shapes=[
            pltpu.VMEM(A_x.shape, _BF16),
            pltpu.VMEM(A_wq.shape, _BF16),
            pltpu.VMEM(A_wo.shape, _BF16),
            pltpu.VMEM(B_w3.shape, _BF16),
            pltpu.VMEM(B_w4.shape, _BF16),
            pltpu.VMEM((_NB, dh, win), _BF16),
            pltpu.VMEM((_NB, dh, win), _BF16),
            pltpu.VMEM((n_heads, _ROWS, dh), _BF16),
            pltpu.SemaphoreType.DMA((4,)),
            pltpu.SemaphoreType.DMA((_NB,)),
            pltpu.SemaphoreType.DMA((_NB,)),
            pltpu.SemaphoreType.DMA((len(_w4_chunks(f)),)),
        ],
        compiler_params=pltpu.CompilerParams(vmem_limit_bytes=64 * 1024 * 1024),
    )(A_x, kt, vt, A_wq, A_wo, B_w3, B_w4)
```

```python
import functools

import jax
import jax.numpy as jnp
from jax import lax
import jax.experimental.pallas as pl
import jax.experimental.pallas.tpu as pltpu

_F32 = jnp.float32
_BF16 = jnp.bfloat16
_EPS = 1e-5
_ROWS = 8
_U = 16
_NT = (((1,), (1,)), ((), ()))

_WQ_ROWS, _WQ_HI = 8, 1024
_WO_ROWS, _WO_HI = 96, 16
_W3_ROWS, _W3_HI = 40, 8
_W4_ROWS, _W4_HI = 64, 16
_KV_HI = 32
_CHUNKS = 8
_W4_GROUPS = (6, 6, 6, 2, 2, 1, 1)


def _layernorm(x):
    m = jnp.mean(x, axis=-1, keepdims=True)
    xc = x - m
    v = jnp.mean(xc * xc, axis=-1, keepdims=True)
    return xc / jnp.sqrt(v + _EPS)


class _Block:
    def __init__(self, src, dst, sem, n_hi, axis=0):
        self.src, self.dst, self.sem, self.n_hi, self.axis = src, dst, sem, n_hi, axis

    def _piece(self, a, n):
        idx = (pl.ds(a, n),) if self.axis == 0 else (slice(None), pl.ds(a, n))
        return pltpu.make_async_copy(self.src.at[idx], self.dst.at[idx], self.sem)

    def start(self):
        n = self.dst.shape[self.axis]
        self._piece(0, self.n_hi).start(priority=0)
        self._piece(self.n_hi, n - self.n_hi).start(priority=1)

    def wait(self):
        pltpu.make_async_copy(self.dst, self.dst, self.sem).wait()


def _rows(i, n):
    return pl.ds(i * n if isinstance(i, int) else pl.multiple_of(i * n, 8), n)


def _kernel(x_hbm, kt_hbm, vt_hbm, wq_hbm, wo_hbm, w3_hbm, w4_hbm, o_ref,
            x_buf, wq_buf, wo_buf, w3_buf, w4_buf, k_buf, v_buf, q_scr, s_scr, p_scr,
            x_sem, sem, w4_sem, *, n_heads, dh, sk, win):
    start = sk - win
    scale = dh ** -0.5
    d = x_buf.shape[-1]
    f = w3_buf.shape[1]
    cb = win // _U
    cw = win // _CHUNKS
    n_wq = d // _WQ_ROWS
    n_wo = n_heads * dh // _WO_ROWS
    n_w4 = f // _W4_ROWS

    def wq_blk(b, j):
        r = _rows(b, _WQ_ROWS)
        return _Block(wq_hbm.at[r], wq_buf.at[r], sem.at[j], _WQ_HI, axis=1)

    def wo_blk(b, j):
        r = _rows(b, _WO_ROWS)
        return _Block(wo_hbm.at[r], wo_buf.at[r], sem.at[j], _WO_HI)

    def k_blk(h, j):
        return _Block(kt_hbm.at[0, h, :, pl.ds(start + j * cb, cb)],
                      k_buf.at[h % 2, :, pl.ds(j * cb, cb)], sem.at[j], _KV_HI)

    def v_blk(h, j):
        return _Block(vt_hbm.at[0, h, :, pl.ds(start + j * cb, cb)],
                      v_buf.at[h % 2, :, pl.ds(j * cb, cb)], sem.at[j], _KV_HI)

    def w3_blk(j):
        r = _rows(j, _W3_ROWS)
        return _Block(w3_hbm.at[r], w3_buf.at[r], sem.at[j], _W3_HI)

    def w4_blk(j):
        r = _rows(j, _W4_ROWS)
        return _Block(w4_hbm.at[r], w4_buf.at[r], w4_sem.at[j], _W4_HI)

    x_cp = pltpu.make_async_copy(x_hbm, x_buf, x_sem.at[0])
    x_cp.start()
    for j in range(_U):
        wq_blk(j, j).start()

    x_cp.wait()
    x = jnp.broadcast_to(x_buf[0].astype(_F32), (_ROWS, d))
    xn = _layernorm(x).astype(_BF16)

    def wq_tick(b, c):
        j = b % _U
        wq_blk(b, j).wait()
        wq_blk(b + _U, j).start()
        return c
    lax.fori_loop(0, n_wq - _U, wq_tick, 0)

    def wq_wo_tick(j, c):
        wq_blk(n_wq - _U + j, j).wait()
        wo_blk(j, j).start()
        return c
    lax.fori_loop(0, _U, wq_wo_tick, 0)

    per_pair = (n_wo - _U) // (n_heads // 2)

    def wo_ticks(i, c):
        for t in range(per_pair):
            b = i * per_pair + t
            j = b % _U
            wo_blk(b, j).wait()
            wo_blk(b + _U, j).start()
            if t == 0:
                col = pl.multiple_of(i * (2 * dh), 128)
                qq = jnp.dot(xn, wq_buf[:, pl.ds(col, 2 * dh)],
                             preferred_element_type=_F32).astype(_BF16)
                q_scr[2 * i] = qq[:, :dh]
                q_scr[2 * i + 1] = qq[:, dh:]
        return c
    lax.fori_loop(0, n_heads // 2, wo_ticks, 0)

    for j in range(_U):
        wo_blk(n_wo - _U + j, j).wait()
        k_blk(0, j).start()
    for j in range(_U):
        k_blk(0, j).wait()
        v_blk(0, j).start()

    def phase_a(h, start_next):
        m = l = None
        for j in range(_U):
            v_blk(h, j).wait()
            start_next(j)
            if j < _CHUNKS:
                cols = slice(j * cw, (j + 1) * cw)
                s = jnp.dot(q_scr[h], k_buf[h % 2, :, cols],
                            preferred_element_type=_F32) * scale
                s_scr[:, cols] = s
                for c in range(cw // 128):
                    sc = s[:, c * 128:(c + 1) * 128]
                    m = sc if m is None else jnp.maximum(m, sc)
            elif j == _CHUNKS:
                m = jnp.max(m, axis=-1, keepdims=True)
            elif j == _CHUNKS + 1:
                p = jnp.exp(s_scr[...] - m)
                p_scr[...] = p.astype(_BF16)
                l = jnp.sum(p, axis=-1, keepdims=True)
        return l

    def phase_b(h, l, attn, wait_cur, start_next):
        o = None
        for j in range(_U):
            wait_cur(j)
            start_next(j)
            if j < _CHUNKS:
                cols = slice(j * cw, (j + 1) * cw)
                oj = lax.dot_general(p_scr[:, cols], v_buf[h % 2, :, cols], _NT,
                                     preferred_element_type=_F32)
                o = oj if o is None else o + oj
            elif j == _CHUNKS:
                attn = attn + jnp.dot((o / l).astype(_BF16), wo_buf[_rows(h, dh), :],
                                      preferred_element_type=_F32)
        return attn

    def head(h, attn):
        l = phase_a(h, lambda j: k_blk(h + 1, j).start())
        return phase_b(h, l, attn,
                       lambda j: k_blk(h + 1, j).wait(),
                       lambda j: v_blk(h + 1, j).start())

    attn = lax.fori_loop(0, n_heads - 1, head, jnp.zeros(x.shape, _F32))

    def start_w4(j):
        for b in range(j * n_w4 // _U, (j + 1) * n_w4 // _U):
            w4_blk(b).start()

    last = n_heads - 1
    l = phase_a(last, lambda j: w3_blk(j).start())
    attn = phase_b(last, l, attn, lambda j: w3_blk(j).wait(), start_w4)

    hres = x + attn
    y = _layernorm(hres)
    z = _layernorm(y).astype(_BF16)
    g = jax.nn.gelu(jnp.dot(z, w3_buf[...], preferred_element_type=_F32),
                    approximate=True).astype(_BF16)
    out = hres + y
    b = 0
    for n in _W4_GROUPS:
        for i in range(n):
            w4_blk(b + i).wait()
        r0, r1 = b * _W4_ROWS, (b + n) * _W4_ROWS
        out = out + jnp.dot(g[:, r0:r1], w4_buf[r0:r1, :], preferred_element_type=_F32)
        b += n
    o_ref[0] = out[0:1].astype(o_ref.dtype)


@jax.jit
def pallas_sequential_preLN__sliding_block_cached__mixer_s_mlp__decode_kernel(
    A_x: jax.Array,
    A_k_cache: jax.Array,
    A_v_cache: jax.Array,
    A_wq: jax.Array,
    A_wo: jax.Array,
    B_x: jax.Array,
    B_w1: jax.Array,
    B_w2: jax.Array,
    B_w3: jax.Array,
    B_w4: jax.Array,
):
    b, sq, d = A_x.shape
    _, n_heads, sk, dh = A_k_cache.shape
    win = min(4096, max(256, sk // 4))
    f = B_w3.shape[1]
    assert (b, sq, d, n_heads, dh, win, f) == (1, 1, 640, 32, 192, 4096, 1536)
    assert d == _U * _W3_ROWS and f == sum(_W4_GROUPS) * _W4_ROWS

    kt = jnp.swapaxes(A_k_cache, 2, 3)
    vt = jnp.swapaxes(A_v_cache, 2, 3)

    any_spec = pl.BlockSpec(memory_space=pl.ANY)
    return pl.pallas_call(
        functools.partial(_kernel, n_heads=n_heads, dh=dh, sk=sk, win=win),
        in_specs=[any_spec] * 7,
        out_specs=pl.BlockSpec(memory_space=pltpu.VMEM),
        out_shape=jax.ShapeDtypeStruct(A_x.shape, A_x.dtype),
        scratch_shapes=[
            pltpu.VMEM(A_x.shape, _BF16),
            pltpu.VMEM(A_wq.shape, _BF16),
            pltpu.VMEM(A_wo.shape, _BF16),
            pltpu.VMEM(B_w3.shape, _BF16),
            pltpu.VMEM(B_w4.shape, _BF16),
            pltpu.VMEM((2, dh, win), _BF16),
            pltpu.VMEM((2, dh, win), _BF16),
            pltpu.VMEM((n_heads, _ROWS, dh), _BF16),
            pltpu.VMEM((_ROWS, win), _F32),
            pltpu.VMEM((_ROWS, win), _BF16),
            pltpu.SemaphoreType.DMA((1,)),
            pltpu.SemaphoreType.DMA((_U,)),
            pltpu.SemaphoreType.DMA((f // _W4_ROWS,)),
        ],
        compiler_params=pltpu.CompilerParams(
            vmem_limit_bytes=64 * 1024 * 1024,
            disable_bounds_checks=True,
            disable_semaphore_checks=True,
        ),
    )(A_x, kt, vt, A_wq, A_wo, B_w3, B_w4)
```

```python
import functools

import jax
import jax.numpy as jnp
from jax import lax
import jax.experimental.pallas as pl
import jax.experimental.pallas.tpu as pltpu

_F32 = jnp.float32
_BF16 = jnp.bfloat16
_EPS = 1e-5
_ROWS = 8
_NT = (((1,), (1,)), ((), ()))

_LOOK_HI = 16
_LOOK_LO = 32
_KV_HI = 32
_STRIDE = 3
_CHUNKS = 8
_GQ, _CQ, _HQ = 10, 768, 2
_GO, _HO = 8, 2
_G3, _H3 = 4, 1
_G4, _R4, _H4 = 4, 16, 1
_W3_SLICES = 6
_W4_STEPS = (8, 8, 4, 2, 2)


def _layernorm(x):
    m = jnp.mean(x, axis=-1, keepdims=True)
    xc = x - m
    v = jnp.mean(xc * xc, axis=-1, keepdims=True)
    return xc / jnp.sqrt(v + _EPS)


def _mul(i, n, align):
    return i * n if isinstance(i, int) else pl.multiple_of(i * n, align)


class _Block:
    def __init__(self, src, dst, sem, n_hi):
        self.src, self.dst, self.sem, self.n_hi = src, dst, sem, n_hi

    def _piece(self, a, n):
        return pltpu.make_async_copy(
            self.src.at[pl.ds(a, n)], self.dst.at[pl.ds(a, n)], self.sem)

    def hi(self):
        self._piece(0, self.n_hi).start(priority=0)

    def lo(self):
        self._piece(self.n_hi, self.dst.shape[0] - self.n_hi).start(priority=1)

    def wait(self):
        pltpu.make_async_copy(self.dst, self.dst, self.sem).wait()


def _tick(j, n, cur, nxt):
    cur(j).wait()
    ahead = lambda p: cur(p) if p < n else nxt(p - n)
    bh, bl = ahead(j + _LOOK_HI), ahead(j + _LOOK_LO)
    if bh is not None:
        bh.hi()
    if bl is not None:
        bl.lo()


def _kernel(x_hbm, kt_hbm, vt_hbm, wq_hbm, wo_hbm, w3_hbm, w4_hbm, o_ref,
            x_buf, wq_buf, wo_buf, w3_buf, w4_buf, k_buf, v_buf, q_scr, s_scr, p_scr,
            x_sem, q_sem, o_sem, k_sem, v_sem, w3_sem, w4_sem, *, n_heads, dh, sk, win):
    start = sk - win
    scale = dh ** -0.5
    d = x_buf.shape[-1]
    f = w3_buf.shape[-1]
    pr = 2 * dh
    n_pairs = n_heads // 2
    cw = win // _CHUNKS
    ncq = wq_buf.shape[2] // _CQ
    nq, no, n3, n4, nkv = (s.shape[0] for s in (q_sem, o_sem, w3_sem, w4_sem, k_sem))

    def wq_blk(b):
        idx = (slice(None), pl.ds(_mul(b // ncq, 8, 8), 8), pl.ds(_mul(b % ncq, _CQ, 128), _CQ))
        return _Block(wq_hbm.at[idx], wq_buf.at[idx], q_sem.at[b], _HQ)

    def wo_blk(b):
        idx = (slice(None), pl.ds(_mul(b, 8, 8), 8))
        return _Block(wo_hbm.at[idx], wo_buf.at[idx], o_sem.at[b], _HO)

    def mlp_blk(b):
        if b < n3:
            idx = (slice(None), pl.ds(b * 8, 8))
            return _Block(w3_hbm.at[idx], w3_buf.at[idx], w3_sem.at[b], _H3)
        if b < n3 + n4:
            idx = (slice(None), pl.ds((b - n3) * _R4, _R4))
            return _Block(w4_hbm.at[idx], w4_buf.at[idx], w4_sem.at[b - n3], _H4)
        return None

    def kv_stream(src, buf, sem, i):
        def blk(j):
            c, hh = divmod(j, 2)
            return _Block(src.at[pl.ds(_mul(i, pr, 8) + hh * dh, dh), pl.ds(start + c * 128, 128)],
                          buf.at[i % 2, pl.ds(hh * dh, dh), pl.ds(c * 128, 128)],
                          sem.at[j], _KV_HI)
        return blk

    k_of = functools.partial(kv_stream, kt_hbm, k_buf, k_sem)
    v_of = functools.partial(kv_stream, vt_hbm, v_buf, v_sem)

    x_cp = pltpu.make_async_copy(x_hbm, x_buf, x_sem.at[0])
    x_cp.start()
    for b in range(_LOOK_LO):
        if b < _LOOK_HI:
            wq_blk(b).hi()
        wq_blk(b).lo()
    x_cp.wait()
    x = jnp.broadcast_to(x_buf[0].astype(_F32), (_ROWS, d))
    xn = _layernorm(x).astype(_BF16)

    def wq_tick(b, c):
        wq_blk(b).wait()
        wq_blk(b + _LOOK_HI).hi()
        wq_blk(b + _LOOK_LO).lo()
        return c
    lax.fori_loop(0, nq - _LOOK_LO, wq_tick, 0)
    for j in range(nq - _LOOK_LO, nq):
        _tick(j, nq, wq_blk, wo_blk)

    per_pair = (no - _LOOK_LO) // n_pairs

    def wo_ticks(i, c):
        for t in range(per_pair):
            b = i * per_pair + t
            wo_blk(b).wait()
            wo_blk(b + _LOOK_HI).hi()
            wo_blk(b + _LOOK_LO).lo()
            if t < pr // 128:
                col = pl.multiple_of(i * pr + t * 128, 128)
                w = wq_buf[:, :, pl.ds(col, 128)].reshape(d, 128)
                q_scr[i, :, t * 128:(t + 1) * 128] = jnp.dot(
                    xn, w, preferred_element_type=_F32).astype(_BF16)
        return c
    lax.fori_loop(0, n_pairs, wo_ticks, 0)
    for j in range(per_pair * n_pairs, no):
        _tick(j, no, wo_blk, k_of(0))

    n_pv = 2 * _CHUNKS + 2

    def pv_slice(j, i, l, o, attn):
        if j < 2 * _CHUNKS:
            hh, c = divmod(j, _CHUNKS)
            cols = slice(c * cw, (c + 1) * cw)
            oj = lax.dot_general(p_scr[hh, :, cols], v_buf[i % 2, hh * dh:(hh + 1) * dh, cols],
                                 _NT, preferred_element_type=_F32)
            o[hh] = oj if o[hh] is None else o[hh] + oj
        elif j < n_pv:
            hh = j - 2 * _CHUNKS
            ppg = wo_buf.shape[1] // pr
            w = wo_buf[i // ppg, pl.ds(_mul(i % ppg, pr, 64) + hh * dh, dh), :]
            attn = attn + jnp.dot((o[hh] / l[hh]).astype(_BF16), w,
                                  preferred_element_type=_F32)
        return attn

    def k_phase(i, l, attn):
        o = [None, None]
        for j in range(nkv):
            _tick(j, nkv, k_of(i), v_of(i))
            if l is not None and j % _STRIDE == 0:
                attn = pv_slice(j // _STRIDE, i - 1, l, o, attn)
        return attn

    def v_phase(i, nxt):
        m = [None, None]
        l = [None, None]
        qh = None
        for j in range(nkv):
            _tick(j, nkv, v_of(i), nxt)
            if j % _STRIDE:
                continue
            jj = j // _STRIDE
            if jj == 0:
                qq = q_scr[i]
                qh = [qq[:, :dh], qq[:, dh:]]
            if jj < 2 * _CHUNKS:
                hh, c = divmod(jj, _CHUNKS)
                cols = slice(c * cw, (c + 1) * cw)
                s = jnp.dot(qh[hh], k_buf[i % 2, hh * dh:(hh + 1) * dh, cols],
                            preferred_element_type=_F32) * scale
                s_scr[hh, :, cols] = s
                for c2 in range(cw // 128):
                    sc = s[:, c2 * 128:(c2 + 1) * 128]
                    m[hh] = sc if m[hh] is None else jnp.maximum(m[hh], sc)
            elif jj == 2 * _CHUNKS:
                m = [jnp.max(mm, axis=-1, keepdims=True) for mm in m]
            elif jj <= 2 * _CHUNKS + 2:
                hh = jj - (2 * _CHUNKS + 1)
                p = jnp.exp(s_scr[hh] - m[hh])
                p_scr[hh] = p.astype(_BF16)
                l[hh] = jnp.sum(p, axis=-1, keepdims=True)
        return l

    attn = jnp.zeros(x.shape, _F32)
    k_phase(0, None, attn)

    def pair(i, attn):
        l = v_phase(i, k_of(i + 1))
        return k_phase(i + 1, l, attn)

    last = n_pairs - 1
    attn = lax.fori_loop(0, last, pair, attn)
    l = v_phase(last, mlp_blk)

    no_more = lambda b: None
    o = [None, None]
    out = y = z = None
    for j in range(n3):
        _tick(j, n3 + n4, mlp_blk, no_more)
        if 2 * j < n_pv:
            attn = pv_slice(2 * j, last, l, o, attn)
            attn = pv_slice(2 * j + 1, last, l, o, attn)
        elif out is None:
            hres = x + attn
            y = _layernorm(hres)
            out = hres + y
        elif z is None:
            z = _layernorm(y).astype(_BF16)

    rg = w4_buf.shape[1]
    offs = [sum(_W4_STEPS[:k]) * _R4 for k in range(len(_W4_STEPS) + 1)]
    fs = f // _W3_SLICES
    acts, gs, gcol = [], None, None
    b = n3
    for step, n in enumerate(_W4_STEPS):
        for t in range(n):
            if step == 0 and t < _W3_SLICES:
                w = w3_buf[:, :, t * fs:(t + 1) * fs].reshape(d, fs)
                a = jnp.dot(z, w, preferred_element_type=_F32)
                acts.append(jax.nn.gelu(a, approximate=True).astype(_BF16))
            elif step == 0 and t == _W3_SLICES:
                g = jnp.concatenate(acts, axis=1)
                gs = [jnp.concatenate([g[:, k * rg + r0:k * rg + r1] for k in range(_G4)], axis=1)
                      for r0, r1 in zip(offs[:-1], offs[1:])]
                nl = gs[-1].shape[1]
                eye = (lax.broadcasted_iota(jnp.int32, (nl, nl), 0)
                       == lax.broadcasted_iota(jnp.int32, (nl, nl), 1))
                diag = jnp.where(eye, jnp.broadcast_to(gs[-1][0:1].astype(_F32), (nl, nl)), 0.0)
                gcol = jnp.dot(diag.astype(_BF16), jnp.ones((nl, 128), _BF16),
                               preferred_element_type=_F32)
            _tick(b, n3 + n4, mlp_blk, no_more)
            b += 1
        r0, r1 = offs[step], offs[step + 1]
        w = w4_buf[:, r0:r1, :].reshape(_G4 * (r1 - r0), d)
        if step < len(_W4_STEPS) - 1:
            out = out + jnp.dot(gs[step], w, preferred_element_type=_F32)
        else:
            prod = w.astype(_F32) * jnp.concatenate([gcol] * (d // 128), axis=1)
            out = out[0:1] + jnp.sum(prod, axis=0, keepdims=True)
    o_ref[0] = out.astype(o_ref.dtype)


@jax.jit
def pallas_sequential_preLN__sliding_block_cached__mixer_s_mlp__decode_kernel(
    A_x: jax.Array,
    A_k_cache: jax.Array,
    A_v_cache: jax.Array,
    A_wq: jax.Array,
    A_wo: jax.Array,
    B_x: jax.Array,
    B_w1: jax.Array,
    B_w2: jax.Array,
    B_w3: jax.Array,
    B_w4: jax.Array,
):
    b, sq, d = A_x.shape
    _, n_heads, sk, dh = A_k_cache.shape
    win = min(4096, max(256, sk // 4))
    f = B_w3.shape[1]
    assert (b, sq, d, n_heads, dh, win, f) == (1, 1, 640, 32, 192, 4096, 1536)
    assert f == _G4 * _R4 * sum(_W4_STEPS)

    kt = jnp.swapaxes(A_k_cache, 2, 3).reshape(n_heads * dh, sk)
    vt = jnp.swapaxes(A_v_cache, 2, 3).reshape(n_heads * dh, sk)
    grouped = lambda w, g: w.reshape(g, w.shape[0] // g, w.shape[1])
    wq, wo = grouped(A_wq, _GQ), grouped(A_wo, _GO)
    w3, w4 = grouped(B_w3, _G3), grouped(B_w4, _G4)

    any_spec = pl.BlockSpec(memory_space=pl.ANY)
    dma = pltpu.SemaphoreType.DMA
    n_kv = 2 * (win // 128)
    return pl.pallas_call(
        functools.partial(_kernel, n_heads=n_heads, dh=dh, sk=sk, win=win),
        in_specs=[any_spec] * 7,
        out_specs=pl.BlockSpec(memory_space=pltpu.VMEM),
        out_shape=jax.ShapeDtypeStruct(A_x.shape, A_x.dtype),
        scratch_shapes=[
            pltpu.VMEM(A_x.shape, _BF16),
            pltpu.VMEM(wq.shape, _BF16),
            pltpu.VMEM(wo.shape, _BF16),
            pltpu.VMEM(w3.shape, _BF16),
            pltpu.VMEM(w4.shape, _BF16),
            pltpu.VMEM((2, 2 * dh, win), _BF16),
            pltpu.VMEM((2, 2 * dh, win), _BF16),
            pltpu.VMEM((n_heads // 2, _ROWS, 2 * dh), _BF16),
            pltpu.VMEM((2, _ROWS, win), _F32),
            pltpu.VMEM((2, _ROWS, win), _BF16),
            dma((1,)),
            dma((wq.shape[1] // 8 * (wq.shape[2] // _CQ),)),
            dma((wo.shape[1] // 8,)),
            dma((n_kv,)),
            dma((n_kv,)),
            dma((w3.shape[1] // 8,)),
            dma((w4.shape[1] // _R4,)),
        ],
        compiler_params=pltpu.CompilerParams(
            vmem_limit_bytes=64 * 1024 * 1024,
            disable_bounds_checks=True,
            disable_semaphore_checks=True,
        ),
    )(A_x, kt, vt, wq, wo, w3, w4)
```

```python
import functools

import jax
import jax.numpy as jnp
from jax import lax
import jax.experimental.pallas as pl
import jax.experimental.pallas.tpu as pltpu

_F32 = jnp.float32
_BF16 = jnp.bfloat16
_EPS = 1e-5
_ROWS = 8
_NT = (((1,), (1,)), ((), ()))

_LOOK_HI = 14
_LOOK_LO = 32
_KV_HI = 32
_STRIDE = 3
_CHUNKS = 8
_GQ, _CQ, _HQ = 10, 768, 2
_GO, _HO = 8, 2
_G3, _H3 = 4, 1
_G4, _R4, _H4 = 4, 16, 1
_W3_SLICES = 6
_W4_STEPS = (8, 8, 5, 1, 1, 1)
_VPU_STEPS = 3
_RING = 64


def _layernorm(x):
    m = jnp.mean(x, axis=-1, keepdims=True)
    xc = x - m
    v = jnp.mean(xc * xc, axis=-1, keepdims=True)
    return xc / jnp.sqrt(v + _EPS)


def _mul(i, n, align):
    return i * n if isinstance(i, int) else pl.multiple_of(i * n, align)


class _Block:
    def __init__(self, src, dst, sem, n_hi):
        self.src, self.dst, self.sem, self.n_hi = src, dst, sem, n_hi

    def _piece(self, a, n):
        return pltpu.make_async_copy(
            self.src.at[pl.ds(a, n)], self.dst.at[pl.ds(a, n)], self.sem)

    def hi(self):
        self._piece(0, self.n_hi).start(priority=0)

    def lo(self):
        self._piece(self.n_hi, self.dst.shape[0] - self.n_hi).start(priority=1)

    def wait(self):
        pltpu.make_async_copy(self.dst, self.dst, self.sem).wait()


def _tick(j, n, cur, nxt):
    cur(j).wait()
    ahead = lambda p: cur(p) if p < n else nxt(p - n)
    bh, bl = ahead(j + _LOOK_HI), ahead(j + _LOOK_LO)
    if bh is not None:
        bh.hi()
    if bl is not None:
        bl.lo()


def _kernel(x_hbm, kt_hbm, vt_hbm, wq_hbm, wo_hbm, w3_hbm, w4_hbm, o_ref,
            x_buf, wq_buf, wo_buf, w3_buf, w4_buf, k_buf, v_buf, q_scr, s_scr, p_scr,
            x_sem, ring, *, n_heads, dh, sk, win):
    start = sk - win
    scale = dh ** -0.5
    d = x_buf.shape[-1]
    f = w3_buf.shape[-1]
    pr = 2 * dh
    n_pairs = n_heads // 2
    cw = win // _CHUNKS
    ncq = wq_buf.shape[2] // _CQ
    nq = wq_buf.shape[1] // 8 * ncq
    no = wo_buf.shape[1] // 8
    n3 = w3_buf.shape[1] // 8
    n4 = w4_buf.shape[1] // _R4
    nkv = 2 * (win // 128)
    assert nkv % _RING == 0 and nq % _RING == 0 and _LOOK_LO < _RING

    def sem(b, after_wo=True):
        return ring.at[(b + (no if after_wo else 0)) % _RING]

    def wq_blk(b):
        idx = (slice(None), pl.ds(_mul(b // ncq, 8, 8), 8), pl.ds(_mul(b % ncq, _CQ, 128), _CQ))
        return _Block(wq_hbm.at[idx], wq_buf.at[idx], sem(b, False), _HQ)

    def wo_blk(b):
        idx = (slice(None), pl.ds(_mul(b, 8, 8), 8))
        return _Block(wo_hbm.at[idx], wo_buf.at[idx], sem(b, False), _HO)

    def mlp_blk(b):
        if b < n3:
            idx = (slice(None), pl.ds(b * 8, 8))
            return _Block(w3_hbm.at[idx], w3_buf.at[idx], sem(b), _H3)
        if b < n3 + n4:
            idx = (slice(None), pl.ds((b - n3) * _R4, _R4))
            return _Block(w4_hbm.at[idx], w4_buf.at[idx], sem(b), _H4)
        return None

    def kv_stream(src, buf, i, after_wo=True):
        def blk(j):
            c, hh = divmod(j, 2)
            return _Block(src.at[pl.ds(_mul(i, pr, 8) + hh * dh, dh), pl.ds(start + c * 128, 128)],
                          buf.at[i % 2, pl.ds(hh * dh, dh), pl.ds(c * 128, 128)],
                          sem(j, after_wo), _KV_HI)
        return blk

    k_of = functools.partial(kv_stream, kt_hbm, k_buf)
    v_of = functools.partial(kv_stream, vt_hbm, v_buf)

    x_cp = pltpu.make_async_copy(x_hbm, x_buf, x_sem.at[0])
    x_cp.start()
    k0_blk = k_of(0, False)
    for b in range(_LOOK_LO):
        if b < _LOOK_HI:
            k0_blk(b).hi()
        k0_blk(b).lo()
    x_cp.wait()
    x = jnp.broadcast_to(x_buf[0].astype(_F32), (_ROWS, d))
    xn = _layernorm(x).astype(_BF16)

    for j in range(nkv):
        _tick(j, nkv, k0_blk, wq_blk)

    def wq_tick(b, c):
        wq_blk(b).wait()
        wq_blk(b + _LOOK_HI).hi()
        wq_blk(b + _LOOK_LO).lo()
        return c
    lax.fori_loop(0, nq - _LOOK_LO, wq_tick, 0)
    for j in range(nq - _LOOK_LO, nq):
        _tick(j, nq, wq_blk, wo_blk)

    per_pair = (no - _LOOK_LO) // n_pairs

    def wo_ticks(i, c):
        for t in range(per_pair):
            b = i * per_pair + t
            wo_blk(b).wait()
            wo_blk(b + _LOOK_HI).hi()
            wo_blk(b + _LOOK_LO).lo()
            if t < pr // 128:
                col = pl.multiple_of(i * pr + t * 128, 128)
                w = wq_buf[:, :, pl.ds(col, 128)].reshape(d, 128)
                q_scr[i, :, t * 128:(t + 1) * 128] = jnp.dot(
                    xn, w, preferred_element_type=_F32).astype(_BF16)
        return c
    lax.fori_loop(0, n_pairs, wo_ticks, 0)
    for j in range(per_pair * n_pairs, no):
        _tick(j, no, wo_blk, v_of(0))

    n_pv = 2 * _CHUNKS + 2

    def pv_slice(j, i, l, o, attn):
        if j < 2 * _CHUNKS:
            hh, c = divmod(j, _CHUNKS)
            cols = slice(c * cw, (c + 1) * cw)
            oj = lax.dot_general(p_scr[hh, :, cols], v_buf[i % 2, hh * dh:(hh + 1) * dh, cols],
                                 _NT, preferred_element_type=_F32)
            o[hh] = oj if o[hh] is None else o[hh] + oj
        elif j < n_pv:
            hh = j - 2 * _CHUNKS
            ppg = wo_buf.shape[1] // pr
            w = wo_buf[i // ppg, pl.ds(_mul(i % ppg, pr, 64) + hh * dh, dh), :]
            attn = attn + jnp.dot((o[hh] / l[hh]).astype(_BF16), w,
                                  preferred_element_type=_F32)
        return attn

    def k_phase(i, l, attn):
        o = [None, None]
        for j in range(nkv):
            _tick(j, nkv, k_of(i), v_of(i))
            if j % _STRIDE == 0:
                attn = pv_slice(j // _STRIDE, i - 1, l, o, attn)
        return attn

    def v_phase(i, nxt):
        m = [None, None]
        l = [None, None]
        qh = None
        for j in range(nkv):
            _tick(j, nkv, v_of(i), nxt)
            if j % _STRIDE:
                continue
            jj = j // _STRIDE
            if jj == 0:
                qq = q_scr[i]
                qh = [qq[:, :dh], qq[:, dh:]]
            if jj < 2 * _CHUNKS:
                hh, c = divmod(jj, _CHUNKS)
                cols = slice(c * cw, (c + 1) * cw)
                s = jnp.dot(qh[hh], k_buf[i % 2, hh * dh:(hh + 1) * dh, cols],
                            preferred_element_type=_F32) * scale
                s_scr[hh, :, cols] = s
                for c2 in range(cw // 128):
                    sc = s[:, c2 * 128:(c2 + 1) * 128]
                    m[hh] = sc if m[hh] is None else jnp.maximum(m[hh], sc)
            elif jj == 2 * _CHUNKS:
                m = [jnp.max(mm, axis=-1, keepdims=True) for mm in m]
            elif jj <= 2 * _CHUNKS + 2:
                hh = jj - (2 * _CHUNKS + 1)
                p = jnp.exp(s_scr[hh] - m[hh])
                p_scr[hh] = p.astype(_BF16)
                l[hh] = jnp.sum(p, axis=-1, keepdims=True)
        return l

    def pair(i, attn):
        l = v_phase(i, k_of(i + 1))
        return k_phase(i + 1, l, attn)

    last = n_pairs - 1
    attn = lax.fori_loop(0, last, pair, jnp.zeros(x.shape, _F32))
    l = v_phase(last, mlp_blk)

    no_more = lambda b: None
    o = [None, None]
    out = y = z = None
    for j in range(n3):
        _tick(j, n3 + n4, mlp_blk, no_more)
        if 2 * j < n_pv:
            attn = pv_slice(2 * j, last, l, o, attn)
            attn = pv_slice(2 * j + 1, last, l, o, attn)
        elif out is None:
            hres = x + attn
            y = _layernorm(hres)
            out = hres + y
        elif z is None:
            z = _layernorm(y).astype(_BF16)

    rg = w4_buf.shape[1]
    offs = [sum(_W4_STEPS[:k]) * _R4 for k in range(len(_W4_STEPS) + 1)]
    fs = f // _W3_SLICES
    n_mxu = len(_W4_STEPS) - _VPU_STEPS
    acts, gs, gcol = [], None, None
    b = n3
    for step, n in enumerate(_W4_STEPS):
        for t in range(n):
            if step == 0 and t < _W3_SLICES:
                w = w3_buf[:, :, t * fs:(t + 1) * fs].reshape(d, fs)
                a = jnp.dot(z, w, preferred_element_type=_F32)
                acts.append(jax.nn.gelu(a, approximate=True).astype(_BF16))
            elif step == 0 and t == _W3_SLICES:
                g = jnp.concatenate(acts, axis=1)
                gs = [jnp.concatenate([g[:, k * rg + r0:k * rg + r1] for k in range(_G4)], axis=1)
                      for r0, r1 in zip(offs[:-1], offs[1:])]
                gl = jnp.concatenate(gs[n_mxu:], axis=1)
                nl = gl.shape[1]
                eye = (lax.broadcasted_iota(jnp.int32, (nl, nl), 0)
                       == lax.broadcasted_iota(jnp.int32, (nl, nl), 1))
                diag = jnp.where(eye, jnp.broadcast_to(gl[0:1].astype(_F32), (nl, nl)), 0.0)
                gcol = jnp.dot(diag.astype(_BF16), jnp.ones((nl, 128), _BF16),
                               preferred_element_type=_F32)
            _tick(b, n3 + n4, mlp_blk, no_more)
            b += 1
        r0, r1 = offs[step], offs[step + 1]
        w = w4_buf[:, r0:r1, :].reshape(_G4 * (r1 - r0), d)
        if step < n_mxu:
            out = out + jnp.dot(gs[step], w, preferred_element_type=_F32)
            if step == n_mxu - 1:
                out = jnp.where(lax.broadcasted_iota(jnp.int32, out.shape, 0) == 0, out, 0.0)
        else:
            g0 = _G4 * (r0 - offs[n_mxu])
            gc = gcol[g0:g0 + w.shape[0]]
            prod = w.astype(_F32) * jnp.concatenate([gc] * (d // 128), axis=1)
            out = out + jnp.sum(prod.reshape(w.shape[0] // _ROWS, _ROWS, d), axis=0)
    out = jnp.sum(out, axis=0, keepdims=True)
    o_ref[0] = out.astype(o_ref.dtype)


@jax.jit
def pallas_sequential_preLN__sliding_block_cached__mixer_s_mlp__decode_kernel(
    A_x: jax.Array,
    A_k_cache: jax.Array,
    A_v_cache: jax.Array,
    A_wq: jax.Array,
    A_wo: jax.Array,
    B_x: jax.Array,
    B_w1: jax.Array,
    B_w2: jax.Array,
    B_w3: jax.Array,
    B_w4: jax.Array,
):
    b, sq, d = A_x.shape
    _, n_heads, sk, dh = A_k_cache.shape
    win = min(4096, max(256, sk // 4))
    f = B_w3.shape[1]
    assert (b, sq, d, n_heads, dh, win, f) == (1, 1, 640, 32, 192, 4096, 1536)
    assert f == _G4 * _R4 * sum(_W4_STEPS)

    kt = jnp.swapaxes(A_k_cache, 2, 3).reshape(n_heads * dh, sk)
    vt = jnp.swapaxes(A_v_cache, 2, 3).reshape(n_heads * dh, sk)
    grouped = lambda w, g: w.reshape(g, w.shape[0] // g, w.shape[1])
    wq, wo = grouped(A_wq, _GQ), grouped(A_wo, _GO)
    w3, w4 = grouped(B_w3, _G3), grouped(B_w4, _G4)

    any_spec = pl.BlockSpec(memory_space=pl.ANY)
    return pl.pallas_call(
        functools.partial(_kernel, n_heads=n_heads, dh=dh, sk=sk, win=win),
        in_specs=[any_spec] * 7,
        out_specs=pl.BlockSpec(memory_space=pltpu.VMEM),
        out_shape=jax.ShapeDtypeStruct(A_x.shape, A_x.dtype),
        scratch_shapes=[
            pltpu.VMEM(A_x.shape, _BF16),
            pltpu.VMEM(wq.shape, _BF16),
            pltpu.VMEM(wo.shape, _BF16),
            pltpu.VMEM(w3.shape, _BF16),
            pltpu.VMEM(w4.shape, _BF16),
            pltpu.VMEM((2, 2 * dh, win), _BF16),
            pltpu.VMEM((2, 2 * dh, win), _BF16),
            pltpu.VMEM((n_heads // 2, _ROWS, 2 * dh), _BF16),
            pltpu.VMEM((2, _ROWS, win), _F32),
            pltpu.VMEM((2, _ROWS, win), _BF16),
            pltpu.SemaphoreType.DMA((1,)),
            pltpu.SemaphoreType.DMA((_RING,)),
        ],
        compiler_params=pltpu.CompilerParams(
            vmem_limit_bytes=64 * 1024 * 1024,
            disable_bounds_checks=True,
            disable_semaphore_checks=True,
        ),
    )(A_x, kt, vt, wq, wo, w3, w4)
```

```python
import functools

import jax
import jax.numpy as jnp
from jax import lax
import jax.experimental.pallas as pl
import jax.experimental.pallas.tpu as pltpu

_F32 = jnp.float32
_BF16 = jnp.bfloat16
_EPS = 1e-5
_ROWS = 8
_NT = (((1,), (1,)), ((), ()))

_LOOK_HI = 14
_LOOK_LO = 32
_KV_HI = 32
_STRIDE = 3
_CHUNKS = 8
_GQ, _CQ, _HQ = 10, 768, 2
_GO, _HO = 8, 2
_G3, _H3 = 4, 1
_G4, _R4, _H4 = 4, 16, 1
_W3_SLICES = 6
_W4_STEPS = (8, 8, 5, 1, 1, 1)
_VPU_STEPS = 3
_X_TICK = 24
_RING = 64


def _layernorm(x):
    m = jnp.mean(x, axis=-1, keepdims=True)
    xc = x - m
    v = jnp.mean(xc * xc, axis=-1, keepdims=True)
    return xc / jnp.sqrt(v + _EPS)


def _mul(i, n, align):
    return i * n if isinstance(i, int) else pl.multiple_of(i * n, align)


class _Block:
    def __init__(self, src, dst, sem, n_hi):
        self.src, self.dst, self.sem, self.n_hi = src, dst, sem, n_hi

    def _piece(self, a, n):
        return pltpu.make_async_copy(
            self.src.at[pl.ds(a, n)], self.dst.at[pl.ds(a, n)], self.sem)

    def hi(self):
        self._piece(0, self.n_hi).start(priority=0)

    def lo(self):
        self._piece(self.n_hi, self.dst.shape[0] - self.n_hi).start(priority=1)

    def wait(self):
        pltpu.make_async_copy(self.dst, self.dst, self.sem).wait()


def _tick(j, n, cur, nxt):
    cur(j).wait()
    ahead = lambda p: cur(p) if p < n else nxt(p - n)
    bh, bl = ahead(j + _LOOK_HI), ahead(j + _LOOK_LO)
    if bh is not None:
        bh.hi()
    if bl is not None:
        bl.lo()


def _kernel(x_hbm, kt_hbm, vt_hbm, wq_hbm, wo_hbm, w3_hbm, w4_hbm, o_ref,
            x_buf, wq_buf, wo_buf, w3_buf, w4_buf, k_buf, v_buf, q_scr, s_scr, p_scr,
            x_sem, ring, *, n_heads, dh, sk, win):
    start = sk - win
    scale = dh ** -0.5
    d = x_buf.shape[-1]
    f = w3_buf.shape[-1]
    pr = 2 * dh
    n_pairs = n_heads // 2
    cw = win // _CHUNKS
    ncq = wq_buf.shape[2] // _CQ
    nq = wq_buf.shape[1] // 8 * ncq
    no = wo_buf.shape[1] // 8
    n3 = w3_buf.shape[1] // 8
    n4 = w4_buf.shape[1] // _R4
    nkv = 2 * (win // 128)
    assert nkv % _RING == 0 and nq % _RING == 0 and _LOOK_LO < _RING

    def sem(b, after_wo=True):
        return ring.at[(b + (no if after_wo else 0)) % _RING]

    def wq_blk(b):
        idx = (slice(None), pl.ds(_mul(b // ncq, 8, 8), 8), pl.ds(_mul(b % ncq, _CQ, 128), _CQ))
        return _Block(wq_hbm.at[idx], wq_buf.at[idx], sem(b, False), _HQ)

    def wo_blk(b):
        idx = (slice(None), pl.ds(_mul(b, 8, 8), 8))
        return _Block(wo_hbm.at[idx], wo_buf.at[idx], sem(b, False), _HO)

    def mlp_blk(b):
        if b < n3:
            idx = (slice(None), pl.ds(b * 8, 8))
            return _Block(w3_hbm.at[idx], w3_buf.at[idx], sem(b), _H3)
        if b < n3 + n4:
            idx = (slice(None), pl.ds((b - n3) * _R4, _R4))
            return _Block(w4_hbm.at[idx], w4_buf.at[idx], sem(b), _H4)
        return None

    def kv_stream(src, buf, i, after_wo=True):
        def blk(j):
            c, hh = divmod(j, 2)
            return _Block(src.at[pl.ds(_mul(i, pr, 8) + hh * dh, dh), pl.ds(start + c * 128, 128)],
                          buf.at[i % 2, pl.ds(hh * dh, dh), pl.ds(c * 128, 128)],
                          sem(j, after_wo), _KV_HI)
        return blk

    k_of = functools.partial(kv_stream, kt_hbm, k_buf)
    v_of = functools.partial(kv_stream, vt_hbm, v_buf)

    x_cp = pltpu.make_async_copy(x_hbm, x_buf, x_sem.at[0])
    x_cp.start()
    k0_blk = k_of(0, False)
    for b in range(_LOOK_LO):
        if b < _LOOK_HI:
            k0_blk(b).hi()
        k0_blk(b).lo()
    x = xn = None
    for j in range(nkv):
        if j == _X_TICK:
            x_cp.wait()
            x = jnp.broadcast_to(x_buf[0].astype(_F32), (_ROWS, d))
            xn = _layernorm(x).astype(_BF16)
        _tick(j, nkv, k0_blk, wq_blk)

    def wq_tick(b, c):
        wq_blk(b).wait()
        wq_blk(b + _LOOK_HI).hi()
        wq_blk(b + _LOOK_LO).lo()
        return c
    lax.fori_loop(0, nq - _LOOK_LO, wq_tick, 0)
    for j in range(nq - _LOOK_LO, nq):
        _tick(j, nq, wq_blk, wo_blk)

    per_pair = (no - _LOOK_LO) // n_pairs

    def wo_ticks(i, c):
        for t in range(per_pair):
            b = i * per_pair + t
            wo_blk(b).wait()
            wo_blk(b + _LOOK_HI).hi()
            wo_blk(b + _LOOK_LO).lo()
            if t < pr // 128:
                col = pl.multiple_of(i * pr + t * 128, 128)
                w = wq_buf[:, :, pl.ds(col, 128)].reshape(d, 128)
                q_scr[i, :, t * 128:(t + 1) * 128] = jnp.dot(
                    xn, w, preferred_element_type=_F32).astype(_BF16)
        return c
    lax.fori_loop(0, n_pairs, wo_ticks, 0)
    for j in range(per_pair * n_pairs, no):
        _tick(j, no, wo_blk, v_of(0))

    n_pv = 2 * _CHUNKS + 2

    def pv_slice(j, i, l, o, attn):
        if j < 2 * _CHUNKS:
            hh, c = divmod(j, _CHUNKS)
            cols = slice(c * cw, (c + 1) * cw)
            oj = lax.dot_general(p_scr[hh, :, cols], v_buf[i % 2, hh * dh:(hh + 1) * dh, cols],
                                 _NT, preferred_element_type=_F32)
            o[hh] = oj if o[hh] is None else oj + o[hh]
        elif j < n_pv:
            hh = j - 2 * _CHUNKS
            ppg = wo_buf.shape[1] // pr
            w = wo_buf[i // ppg, pl.ds(_mul(i % ppg, pr, 64) + hh * dh, dh), :]
            attn = attn + jnp.dot((o[hh] / l[hh]).astype(_BF16), w,
                                  preferred_element_type=_F32)
        return attn

    def k_phase(i, l, attn):
        o = [None, None]
        for j in range(nkv):
            _tick(j, nkv, k_of(i), v_of(i))
            if j % _STRIDE == 0:
                attn = pv_slice(j // _STRIDE, i - 1, l, o, attn)
        return attn

    def v_phase(i, nxt, stride=_STRIDE, after=None):
        m = [None, None]
        l = [None, None]
        qh = None
        for j in range(nkv):
            _tick(j, nkv, v_of(i), nxt)
            if j % stride:
                continue
            jj = j // stride
            if jj == 0:
                qq = q_scr[i]
                qh = [qq[:, :dh], qq[:, dh:]]
            if jj < 2 * _CHUNKS:
                hh, c = divmod(jj, _CHUNKS)
                cols = slice(c * cw, (c + 1) * cw)
                s = jnp.dot(qh[hh], k_buf[i % 2, hh * dh:(hh + 1) * dh, cols],
                            preferred_element_type=_F32) * scale
                s_scr[hh, :, cols] = s
                for c2 in range(cw // 128):
                    sc = s[:, c2 * 128:(c2 + 1) * 128]
                    m[hh] = sc if m[hh] is None else jnp.maximum(m[hh], sc)
            elif jj == 2 * _CHUNKS:
                m = [jnp.max(mm, axis=-1, keepdims=True) for mm in m]
            elif jj <= 2 * _CHUNKS + 2:
                hh = jj - (2 * _CHUNKS + 1)
                p = jnp.exp(s_scr[hh] - m[hh])
                p_scr[hh] = p.astype(_BF16)
                l[hh] = jnp.sum(p, axis=-1, keepdims=True)
            elif after is not None:
                after(j)
        return l

    def pair(i, attn):
        l = v_phase(i, k_of(i + 1))
        return k_phase(i + 1, l, attn)

    last = n_pairs - 1
    attn = lax.fori_loop(0, last, pair, jnp.zeros(x.shape, _F32))

    o = [None, None]
    todo = [hh * _CHUNKS + c for c in range(_CHUNKS) for hh in range(2)]
    todo += [2 * _CHUNKS, 2 * _CHUNKS + 1]

    def early_pv(j):
        if j + 1 >= (nkv // _CHUNKS) * (todo[0] % _CHUNKS + 1):
            pv_slice(todo.pop(0), last, None, o, None)

    l = v_phase(last, mlp_blk, 2, early_pv)

    no_more = lambda b: None
    out = y = z = None
    for j in range(n3):
        _tick(j, n3 + n4, mlp_blk, no_more)
        if todo:
            attn = pv_slice(todo.pop(0), last, l, o, attn)
        elif out is None:
            hres = x + attn
            y = _layernorm(hres)
            out = hres + y
        elif z is None:
            z = _layernorm(y).astype(_BF16)

    rg = w4_buf.shape[1]
    offs = [sum(_W4_STEPS[:k]) * _R4 for k in range(len(_W4_STEPS) + 1)]
    fs = f // _W3_SLICES
    n_mxu = len(_W4_STEPS) - _VPU_STEPS
    acts, gs, gcol = [], None, None
    b = n3
    for step, n in enumerate(_W4_STEPS):
        for t in range(n):
            if step == 0 and t < _W3_SLICES:
                w = w3_buf[:, :, t * fs:(t + 1) * fs].reshape(d, fs)
                a = jnp.dot(z, w, preferred_element_type=_F32)
                acts.append(jax.nn.gelu(a, approximate=True).astype(_BF16))
            elif step == 0 and t == _W3_SLICES:
                g = jnp.concatenate(acts, axis=1)
                gs = [jnp.concatenate([g[:, k * rg + r0:k * rg + r1] for k in range(_G4)], axis=1)
                      for r0, r1 in zip(offs[:-1], offs[1:])]
                gl = jnp.concatenate(gs[n_mxu:], axis=1)
                nl = gl.shape[1]
                eye = (lax.broadcasted_iota(jnp.int32, (nl, nl), 0)
                       == lax.broadcasted_iota(jnp.int32, (nl, nl), 1))
                diag = jnp.where(eye, jnp.broadcast_to(gl[0:1].astype(_F32), (nl, nl)), 0.0)
                gcol = jnp.dot(diag.astype(_BF16), jnp.ones((nl, 128), _BF16),
                               preferred_element_type=_F32)
            _tick(b, n3 + n4, mlp_blk, no_more)
            b += 1
        r0, r1 = offs[step], offs[step + 1]
        w = w4_buf[:, r0:r1, :].reshape(_G4 * (r1 - r0), d)
        if step < n_mxu:
            out = out + jnp.dot(gs[step], w, preferred_element_type=_F32)
            if step == n_mxu - 1:
                out = jnp.where(lax.broadcasted_iota(jnp.int32, out.shape, 0) == 0, out, 0.0)
        else:
            g0 = _G4 * (r0 - offs[n_mxu])
            gc = gcol[g0:g0 + w.shape[0]]
            prod = w.astype(_F32) * jnp.concatenate([gc] * (d // 128), axis=1)
            out = out + jnp.sum(prod.reshape(w.shape[0] // _ROWS, _ROWS, d), axis=0)
    out = jnp.sum(out, axis=0, keepdims=True)
    o_ref[0] = out.astype(o_ref.dtype)


@jax.jit
def pallas_sequential_preLN__sliding_block_cached__mixer_s_mlp__decode_kernel(
    A_x: jax.Array,
    A_k_cache: jax.Array,
    A_v_cache: jax.Array,
    A_wq: jax.Array,
    A_wo: jax.Array,
    B_x: jax.Array,
    B_w1: jax.Array,
    B_w2: jax.Array,
    B_w3: jax.Array,
    B_w4: jax.Array,
):
    b, sq, d = A_x.shape
    _, n_heads, sk, dh = A_k_cache.shape
    win = min(4096, max(256, sk // 4))
    f = B_w3.shape[1]
    assert (b, sq, d, n_heads, dh, win, f) == (1, 1, 640, 32, 192, 4096, 1536)
    assert f == _G4 * _R4 * sum(_W4_STEPS)

    kt = jnp.swapaxes(A_k_cache, 2, 3).reshape(n_heads * dh, sk)
    vt = jnp.swapaxes(A_v_cache, 2, 3).reshape(n_heads * dh, sk)
    grouped = lambda w, g: w.reshape(g, w.shape[0] // g, w.shape[1])
    wq, wo = grouped(A_wq, _GQ), grouped(A_wo, _GO)
    w3, w4 = grouped(B_w3, _G3), grouped(B_w4, _G4)

    any_spec = pl.BlockSpec(memory_space=pl.ANY)
    return pl.pallas_call(
        functools.partial(_kernel, n_heads=n_heads, dh=dh, sk=sk, win=win),
        in_specs=[any_spec] * 7,
        out_specs=pl.BlockSpec(memory_space=pltpu.VMEM),
        out_shape=jax.ShapeDtypeStruct(A_x.shape, A_x.dtype),
        scratch_shapes=[
            pltpu.VMEM(A_x.shape, _BF16),
            pltpu.VMEM(wq.shape, _BF16),
            pltpu.VMEM(wo.shape, _BF16),
            pltpu.VMEM(w3.shape, _BF16),
            pltpu.VMEM(w4.shape, _BF16),
            pltpu.VMEM((2, 2 * dh, win), _BF16),
            pltpu.VMEM((2, 2 * dh, win), _BF16),
            pltpu.VMEM((n_heads // 2, _ROWS, 2 * dh), _BF16),
            pltpu.VMEM((2, _ROWS, win), _F32),
            pltpu.VMEM((2, _ROWS, win), _BF16),
            pltpu.SemaphoreType.DMA((1,)),
            pltpu.SemaphoreType.DMA((_RING,)),
        ],
        compiler_params=pltpu.CompilerParams(
            vmem_limit_bytes=64 * 1024 * 1024,
            disable_bounds_checks=True,
            disable_semaphore_checks=True,
        ),
    )(A_x, kt, vt, wq, wo, w3, w4)
```

```python
import functools

import jax
import jax.numpy as jnp
from jax import lax
import jax.experimental.pallas as pl
import jax.experimental.pallas.tpu as pltpu

_F32 = jnp.float32
_BF16 = jnp.bfloat16
_EPS = 1e-5
_ROWS = 8
_NT = (((1,), (1,)), ((), ()))

_LOOK_HI = 15
_LOOK_LO = 32
_KV_HI = 32
_STRIDE = 3
_CHUNKS = 8
_GQ, _CQ, _HQ = 10, 384, 2
_GO, _HO = 8, 3
_G3, _H3 = 4, 1
_G4, _R4, _H4 = 4, 16, 1
_W3_SLICES = 6
_W4_STEPS = (8, 8, 5, 1, 1, 1)
_VPU_STEPS = 3
_X_TICK = 24
_PRO_LOOP = 2
_RING = 64


def _layernorm(x):
    m = jnp.mean(x, axis=-1, keepdims=True)
    xc = x - m
    v = jnp.mean(xc * xc, axis=-1, keepdims=True)
    return xc / jnp.sqrt(v + _EPS)


def _mul(i, n, align):
    return i * n if isinstance(i, int) else pl.multiple_of(i * n, align)


class _Block:
    def __init__(self, src, dst, sem, n_hi):
        self.src, self.dst, self.sem, self.n_hi = src, dst, sem, n_hi

    def _piece(self, a, n):
        return pltpu.make_async_copy(
            self.src.at[pl.ds(a, n)], self.dst.at[pl.ds(a, n)], self.sem)

    def hi(self):
        self._piece(0, self.n_hi).start(priority=0)

    def lo(self):
        self._piece(self.n_hi, self.dst.shape[0] - self.n_hi).start(priority=1)

    def wait(self):
        pltpu.make_async_copy(self.dst, self.dst, self.sem).wait()


def _tick(j, n, cur, nxt):
    cur(j).wait()
    ahead = lambda p: cur(p) if p < n else nxt(p - n)
    bh, bl = ahead(j + _LOOK_HI), ahead(j + _LOOK_LO)
    if bh is not None:
        bh.hi()
    if bl is not None:
        bl.lo()


def _kernel(x_hbm, kt_hbm, vt_hbm, wq_hbm, wo_hbm, w3_hbm, w4_hbm, o_ref,
            x_buf, wq_buf, wo_buf, w3_buf, w4_buf, k_buf, v_buf, q_scr, s_scr, p_scr,
            x_sem, ring, *, n_heads, dh, sk, win):
    start = sk - win
    scale = dh ** -0.5
    d = x_buf.shape[-1]
    f = w3_buf.shape[-1]
    pr = 2 * dh
    n_pairs = n_heads // 2
    cw = win // _CHUNKS
    ncq = wq_buf.shape[2] // _CQ
    nq = wq_buf.shape[1] // 8 * ncq
    no = wo_buf.shape[1] // 8
    n3 = w3_buf.shape[1] // 8
    n4 = w4_buf.shape[1] // _R4
    nkv = 2 * (win // 128)
    assert nkv % _RING == 0 and nq % _RING == 0 and _LOOK_LO < _RING

    def sem(b, after_wo=True):
        return ring.at[(b + (no if after_wo else 0)) % _RING]

    def wq_blk(b):
        idx = (slice(None), pl.ds(_mul(b // ncq, 8, 8), 8), pl.ds(_mul(b % ncq, _CQ, 128), _CQ))
        return _Block(wq_hbm.at[idx], wq_buf.at[idx], sem(b, False), _HQ)

    def wo_blk(b):
        idx = (slice(None), pl.ds(_mul(b, 8, 8), 8))
        return _Block(wo_hbm.at[idx], wo_buf.at[idx], sem(b, False), _HO)

    def mlp_blk(b):
        if b < n3:
            idx = (slice(None), pl.ds(b * 8, 8))
            return _Block(w3_hbm.at[idx], w3_buf.at[idx], sem(b), _H3)
        if b < n3 + n4:
            idx = (slice(None), pl.ds((b - n3) * _R4, _R4))
            return _Block(w4_hbm.at[idx], w4_buf.at[idx], sem(b), _H4)
        return None

    def kv_stream(src, buf, i, after_wo=True):
        def blk(j):
            col, row = _mul(j // 2, 128, 128), _mul(j % 2, dh, 8)
            return _Block(src.at[pl.ds(_mul(i, pr, 8) + row, dh), pl.ds(start + col, 128)],
                          buf.at[i % 2, pl.ds(row, dh), pl.ds(col, 128)],
                          sem(j, after_wo), _KV_HI)
        return blk

    k_of = functools.partial(kv_stream, kt_hbm, k_buf)
    v_of = functools.partial(kv_stream, vt_hbm, v_buf)

    x_cp = pltpu.make_async_copy(x_hbm, x_buf, x_sem.at[0])
    x_cp.start()
    k0_blk = k_of(0, False)
    if _PRO_LOOP:
        for b in range(_PRO_LOOP):
            k0_blk(b).lo()

        def first(b, c):
            k0_blk(b).hi()
            k0_blk(b + _PRO_LOOP).lo()
            return c
        lax.fori_loop(0, _LOOK_HI, first, 0)
        for b in range(_PRO_LOOP + _LOOK_HI, _LOOK_LO):
            k0_blk(b).lo()
    else:
        for b in range(_LOOK_LO):
            if b < _LOOK_HI:
                k0_blk(b).hi()
            k0_blk(b).lo()
    x = xn = None
    for j in range(nkv):
        if j == _X_TICK:
            x_cp.wait()
            x = jnp.broadcast_to(x_buf[0].astype(_F32), (_ROWS, d))
            xn = _layernorm(x).astype(_BF16)
        _tick(j, nkv, k0_blk, wq_blk)

    def wq_tick(b, c):
        wq_blk(b).wait()
        wq_blk(b + _LOOK_HI).hi()
        wq_blk(b + _LOOK_LO).lo()
        return c
    lax.fori_loop(0, nq - _LOOK_LO, wq_tick, 0)
    for j in range(nq - _LOOK_LO, nq):
        _tick(j, nq, wq_blk, wo_blk)

    per_pair = (no - _LOOK_LO) // n_pairs

    def wo_ticks(i, c):
        for t in range(per_pair):
            b = i * per_pair + t
            wo_blk(b).wait()
            wo_blk(b + _LOOK_HI).hi()
            wo_blk(b + _LOOK_LO).lo()
            if t < pr // 128:
                col = pl.multiple_of(i * pr + t * 128, 128)
                w = wq_buf[:, :, pl.ds(col, 128)].reshape(d, 128)
                q_scr[i, :, t * 128:(t + 1) * 128] = jnp.dot(
                    xn, w, preferred_element_type=_F32).astype(_BF16)
        return c
    lax.fori_loop(0, n_pairs, wo_ticks, 0)
    for j in range(per_pair * n_pairs, no):
        _tick(j, no, wo_blk, v_of(0))

    n_pv = 2 * _CHUNKS + 2

    def pv_slice(j, i, l, o, attn):
        if j < 2 * _CHUNKS:
            hh, c = divmod(j, _CHUNKS)
            cols = slice(c * cw, (c + 1) * cw)
            oj = lax.dot_general(p_scr[hh, :, cols], v_buf[i % 2, hh * dh:(hh + 1) * dh, cols],
                                 _NT, preferred_element_type=_F32)
            o[hh] = oj if o[hh] is None else oj + o[hh]
        elif j < n_pv:
            hh = j - 2 * _CHUNKS
            ppg = wo_buf.shape[1] // pr
            w = wo_buf[i // ppg, pl.ds(_mul(i % ppg, pr, 64) + hh * dh, dh), :]
            attn = attn + jnp.dot((o[hh] / l[hh]).astype(_BF16), w,
                                  preferred_element_type=_F32)
        return attn

    def k_phase(i, l, attn):
        o = [None, None]
        for j in range(nkv):
            _tick(j, nkv, k_of(i), v_of(i))
            if j % _STRIDE == 0:
                attn = pv_slice(j // _STRIDE, i - 1, l, o, attn)
        return attn

    def v_phase(i, nxt, stride=_STRIDE, after=None):
        m = [None, None]
        l = [None, None]
        qh = None
        for j in range(nkv):
            _tick(j, nkv, v_of(i), nxt)
            if j % stride:
                continue
            jj = j // stride
            if jj == 0:
                qq = q_scr[i]
                qh = [qq[:, :dh], qq[:, dh:]]
            if jj < 2 * _CHUNKS:
                hh, c = divmod(jj, _CHUNKS)
                cols = slice(c * cw, (c + 1) * cw)
                s = jnp.dot(qh[hh], k_buf[i % 2, hh * dh:(hh + 1) * dh, cols],
                            preferred_element_type=_F32) * scale
                s_scr[hh, :, cols] = s
                for c2 in range(cw // 128):
                    sc = s[:, c2 * 128:(c2 + 1) * 128]
                    m[hh] = sc if m[hh] is None else jnp.maximum(m[hh], sc)
            elif jj == 2 * _CHUNKS:
                m = [jnp.max(mm, axis=-1, keepdims=True) for mm in m]
            elif jj <= 2 * _CHUNKS + 2:
                hh = jj - (2 * _CHUNKS + 1)
                p = jnp.exp(s_scr[hh] - m[hh])
                p_scr[hh] = p.astype(_BF16)
                l[hh] = jnp.sum(p, axis=-1, keepdims=True)
            elif after is not None:
                after(j)
        return l

    def pair(i, attn):
        l = v_phase(i, k_of(i + 1))
        return k_phase(i + 1, l, attn)

    last = n_pairs - 1
    attn = lax.fori_loop(0, last, pair, jnp.zeros(x.shape, _F32))

    o = [None, None]
    todo = [hh * _CHUNKS + c for c in range(_CHUNKS) for hh in range(2)]
    todo += [2 * _CHUNKS, 2 * _CHUNKS + 1]

    def early_pv(j):
        if todo[0] < 2 * _CHUNKS and j + 1 >= (nkv // _CHUNKS) * (todo[0] % _CHUNKS + 1):
            pv_slice(todo.pop(0), last, None, o, None)

    l = v_phase(last, mlp_blk, 2, early_pv)

    no_more = lambda b: None
    out = y = z = None
    for j in range(n3):
        _tick(j, n3 + n4, mlp_blk, no_more)
        if todo:
            attn = pv_slice(todo.pop(0), last, l, o, attn)
        elif out is None:
            hres = x + attn
            y = _layernorm(hres)
            out = hres + y
        elif z is None:
            z = _layernorm(y).astype(_BF16)

    rg = w4_buf.shape[1]
    offs = [sum(_W4_STEPS[:k]) * _R4 for k in range(len(_W4_STEPS) + 1)]
    fs = f // _W3_SLICES
    n_mxu = len(_W4_STEPS) - _VPU_STEPS
    acts, gs, gcol = [], None, None
    b = n3
    for step, n in enumerate(_W4_STEPS):
        for t in range(n):
            if step == 0 and t < _W3_SLICES:
                w = w3_buf[:, :, t * fs:(t + 1) * fs].reshape(d, fs)
                a = jnp.dot(z, w, preferred_element_type=_F32)
                acts.append(jax.nn.gelu(a, approximate=True).astype(_BF16))
            elif step == 0 and t == _W3_SLICES:
                g = jnp.concatenate(acts, axis=1)
                gs = [jnp.concatenate([g[:, k * rg + r0:k * rg + r1] for k in range(_G4)], axis=1)
                      for r0, r1 in zip(offs[:-1], offs[1:])]
                gl = jnp.concatenate(gs[n_mxu:], axis=1)
                nl = gl.shape[1]
                eye = (lax.broadcasted_iota(jnp.int32, (nl, nl), 0)
                       == lax.broadcasted_iota(jnp.int32, (nl, nl), 1))
                diag = jnp.where(eye, jnp.broadcast_to(gl[0:1].astype(_F32), (nl, nl)), 0.0)
                gcol = jnp.dot(diag.astype(_BF16), jnp.ones((nl, 128), _BF16),
                               preferred_element_type=_F32)
            _tick(b, n3 + n4, mlp_blk, no_more)
            b += 1
        r0, r1 = offs[step], offs[step + 1]
        w = w4_buf[:, r0:r1, :].reshape(_G4 * (r1 - r0), d)
        if step < n_mxu:
            out = out + jnp.dot(gs[step], w, preferred_element_type=_F32)
            if step == n_mxu - 1:
                out = jnp.where(lax.broadcasted_iota(jnp.int32, out.shape, 0) == 0, out, 0.0)
        else:
            g0 = _G4 * (r0 - offs[n_mxu])
            gc = gcol[g0:g0 + w.shape[0]]
            prod = w.astype(_F32) * jnp.concatenate([gc] * (d // 128), axis=1)
            out = out + jnp.sum(prod.reshape(w.shape[0] // _ROWS, _ROWS, d), axis=0)
    out = jnp.sum(out, axis=0, keepdims=True)
    o_ref[0] = out.astype(o_ref.dtype)


@jax.jit
def pallas_sequential_preLN__sliding_block_cached__mixer_s_mlp__decode_kernel(
    A_x: jax.Array,
    A_k_cache: jax.Array,
    A_v_cache: jax.Array,
    A_wq: jax.Array,
    A_wo: jax.Array,
    B_x: jax.Array,
    B_w1: jax.Array,
    B_w2: jax.Array,
    B_w3: jax.Array,
    B_w4: jax.Array,
):
    b, sq, d = A_x.shape
    _, n_heads, sk, dh = A_k_cache.shape
    win = min(4096, max(256, sk // 4))
    f = B_w3.shape[1]
    assert (b, sq, d, n_heads, dh, win, f) == (1, 1, 640, 32, 192, 4096, 1536)
    assert f == _G4 * _R4 * sum(_W4_STEPS)

    kt = jnp.swapaxes(A_k_cache, 2, 3).reshape(n_heads * dh, sk)
    vt = jnp.swapaxes(A_v_cache, 2, 3).reshape(n_heads * dh, sk)
    grouped = lambda w, g: w.reshape(g, w.shape[0] // g, w.shape[1])
    wq, wo = grouped(A_wq, _GQ), grouped(A_wo, _GO)
    w3, w4 = grouped(B_w3, _G3), grouped(B_w4, _G4)

    any_spec = pl.BlockSpec(memory_space=pl.ANY)
    return pl.pallas_call(
        functools.partial(_kernel, n_heads=n_heads, dh=dh, sk=sk, win=win),
        in_specs=[any_spec] * 7,
        out_specs=pl.BlockSpec(memory_space=pltpu.VMEM),
        out_shape=jax.ShapeDtypeStruct(A_x.shape, A_x.dtype),
        scratch_shapes=[
            pltpu.VMEM(A_x.shape, _BF16),
            pltpu.VMEM(wq.shape, _BF16),
            pltpu.VMEM(wo.shape, _BF16),
            pltpu.VMEM(w3.shape, _BF16),
            pltpu.VMEM(w4.shape, _BF16),
            pltpu.VMEM((2, 2 * dh, win), _BF16),
            pltpu.VMEM((2, 2 * dh, win), _BF16),
            pltpu.VMEM((n_heads // 2, _ROWS, 2 * dh), _BF16),
            pltpu.VMEM((2, _ROWS, win), _F32),
            pltpu.VMEM((2, _ROWS, win), _BF16),
            pltpu.SemaphoreType.DMA((1,)),
            pltpu.SemaphoreType.DMA((_RING,)),
        ],
        compiler_params=pltpu.CompilerParams(
            vmem_limit_bytes=64 * 1024 * 1024,
            disable_bounds_checks=True,
            disable_semaphore_checks=True,
        ),
    )(A_x, kt, vt, wq, wo, w3, w4)
```

```python
import functools

import jax
import jax.numpy as jnp
from jax import lax
import jax.experimental.pallas as pl
import jax.experimental.pallas.tpu as pltpu

_F32 = jnp.float32
_BF16 = jnp.bfloat16
_EPS = 1e-5
_ROWS = 8
_NT = (((1,), (1,)), ((), ()))

_LOOK_HI = 15
_LOOK_LO = 32
_KV_HI = 32
_STRIDE = 3
_CHUNKS = 8
_GQ, _CQ, _HQ = 10, 384, 2
_GO, _HO = 8, 3
_G3, _H3 = 4, 1
_G4, _R4, _H4 = 4, 16, 1
_W3_SLICES = 6
_W4_STEPS = (8, 8, 5, 1, 1, 1)
_VPU_STEPS = 3
_X_TICK = 24
_PRO_LO = 2
_HEAD_MAJOR = True
_RING = 64


def _layernorm(x):
    m = jnp.mean(x, axis=-1, keepdims=True)
    xc = x - m
    v = jnp.mean(xc * xc, axis=-1, keepdims=True)
    return xc / jnp.sqrt(v + _EPS)


def _mul(i, n, align):
    return i * n if isinstance(i, int) else pl.multiple_of(i * n, align)


class _Block:
    def __init__(self, src, dst, sem, n_hi):
        self.src, self.dst, self.sem, self.n_hi = src, dst, sem, n_hi

    def _piece(self, a, n):
        return pltpu.make_async_copy(
            self.src.at[pl.ds(a, n)], self.dst.at[pl.ds(a, n)], self.sem)

    def hi(self):
        self._piece(0, self.n_hi).start(priority=0)

    def lo(self):
        self._piece(self.n_hi, self.dst.shape[0] - self.n_hi).start(priority=1)

    def wait(self):
        pltpu.make_async_copy(self.dst, self.dst, self.sem).wait()


def _tick(j, n, cur, nxt):
    cur(j).wait()
    ahead = lambda p: cur(p) if p < n else nxt(p - n)
    bh, bl = ahead(j + _LOOK_HI), ahead(j + _LOOK_LO)
    if bh is not None:
        bh.hi()
    if bl is not None:
        bl.lo()


def _kernel(x_hbm, kt_hbm, vt_hbm, wq_hbm, wo_hbm, w3_hbm, w4_hbm, o_ref,
            x_buf, wq_buf, wo_buf, w3_buf, w4_buf, k_buf, v_buf, q_scr, s_scr, p_scr,
            x_sem, ring, *, n_heads, dh, sk, win):
    start = sk - win
    scale = dh ** -0.5
    d = x_buf.shape[-1]
    f = w3_buf.shape[-1]
    pr = 2 * dh
    n_pairs = n_heads // 2
    cw = win // _CHUNKS
    ncq = wq_buf.shape[2] // _CQ
    nq = wq_buf.shape[1] // 8 * ncq
    no = wo_buf.shape[1] // 8
    n3 = w3_buf.shape[1] // 8
    n4 = w4_buf.shape[1] // _R4
    nkv = 2 * (win // 128)
    assert nkv % _RING == 0 and nq % _RING == 0 and _LOOK_LO < _RING

    def sem(b, after_wo=True):
        return ring.at[(b + (no if after_wo else 0)) % _RING]

    def wq_blk(b):
        idx = (slice(None), pl.ds(_mul(b // ncq, 8, 8), 8), pl.ds(_mul(b % ncq, _CQ, 128), _CQ))
        return _Block(wq_hbm.at[idx], wq_buf.at[idx], sem(b, False), _HQ)

    def wo_blk(b):
        idx = (slice(None), pl.ds(_mul(b, 8, 8), 8))
        return _Block(wo_hbm.at[idx], wo_buf.at[idx], sem(b, False), _HO)

    def mlp_blk(b):
        if b < n3:
            idx = (slice(None), pl.ds(b * 8, 8))
            return _Block(w3_hbm.at[idx], w3_buf.at[idx], sem(b), _H3)
        if b < n3 + n4:
            idx = (slice(None), pl.ds((b - n3) * _R4, _R4))
            return _Block(w4_hbm.at[idx], w4_buf.at[idx], sem(b), _H4)
        return None

    def kv_stream(src, buf, i, after_wo=True):
        def blk(j):
            if _HEAD_MAJOR:
                col, row = _mul(j % (nkv // 2), 128, 128), _mul(j // (nkv // 2), dh, 8)
            else:
                col, row = _mul(j // 2, 128, 128), _mul(j % 2, dh, 8)
            return _Block(src.at[pl.ds(_mul(i, pr, 8) + row, dh), pl.ds(start + col, 128)],
                          buf.at[i % 2, pl.ds(row, dh), pl.ds(col, 128)],
                          sem(j, after_wo), _KV_HI)
        return blk

    k_of = functools.partial(kv_stream, kt_hbm, k_buf)
    v_of = functools.partial(kv_stream, vt_hbm, v_buf)

    x_cp = pltpu.make_async_copy(x_hbm, x_buf, x_sem.at[0])
    x_cp.start()
    k0_blk = k_of(0, False)
    for b in range(_PRO_LO):
        k0_blk(b).lo()

    def first(b, c):
        k0_blk(b).hi()
        k0_blk(b + _PRO_LO).lo()
        return c
    lax.fori_loop(0, _LOOK_HI, first, 0)
    for b in range(_PRO_LO + _LOOK_HI, _LOOK_LO):
        k0_blk(b).lo()
    x = xn = None
    for j in range(nkv):
        if j == _X_TICK:
            x_cp.wait()
            x = jnp.broadcast_to(x_buf[0].astype(_F32), (_ROWS, d))
            xn = _layernorm(x).astype(_BF16)
        _tick(j, nkv, k0_blk, wq_blk)

    def wq_tick(b, c):
        wq_blk(b).wait()
        wq_blk(b + _LOOK_HI).hi()
        wq_blk(b + _LOOK_LO).lo()
        return c
    lax.fori_loop(0, nq - _LOOK_LO, wq_tick, 0)
    for j in range(nq - _LOOK_LO, nq):
        _tick(j, nq, wq_blk, wo_blk)

    per_pair = (no - _LOOK_LO) // n_pairs

    def wo_ticks(i, c):
        for t in range(per_pair):
            b = i * per_pair + t
            wo_blk(b).wait()
            wo_blk(b + _LOOK_HI).hi()
            wo_blk(b + _LOOK_LO).lo()
            if t < pr // 128:
                col = pl.multiple_of(i * pr + t * 128, 128)
                w = wq_buf[:, :, pl.ds(col, 128)].reshape(d, 128)
                q_scr[i, :, t * 128:(t + 1) * 128] = jnp.dot(
                    xn, w, preferred_element_type=_F32).astype(_BF16)
        return c
    lax.fori_loop(0, n_pairs, wo_ticks, 0)
    for j in range(per_pair * n_pairs, no):
        _tick(j, no, wo_blk, v_of(0))

    n_pv = 2 * _CHUNKS + 2

    def pv_slice(j, i, l, o, attn):
        if j < 2 * _CHUNKS:
            hh, c = divmod(j, _CHUNKS)
            cols = slice(c * cw, (c + 1) * cw)
            oj = lax.dot_general(p_scr[hh, :, cols], v_buf[i % 2, hh * dh:(hh + 1) * dh, cols],
                                 _NT, preferred_element_type=_F32)
            o[hh] = oj if o[hh] is None else oj + o[hh]
        elif j < n_pv:
            hh = j - 2 * _CHUNKS
            ppg = wo_buf.shape[1] // pr
            w = wo_buf[i // ppg, pl.ds(_mul(i % ppg, pr, 64) + hh * dh, dh), :]
            attn = attn + jnp.dot((o[hh] / l[hh]).astype(_BF16), w,
                                  preferred_element_type=_F32)
        return attn

    def k_phase(i, l, attn):
        o = [None, None]
        for j in range(nkv):
            _tick(j, nkv, k_of(i), v_of(i))
            if j % _STRIDE == 0:
                attn = pv_slice(j // _STRIDE, i - 1, l, o, attn)
        return attn

    def v_phase(i, nxt, stride=_STRIDE, after=None):
        m = [None, None]
        l = [None, None]
        qh = None
        for j in range(nkv):
            _tick(j, nkv, v_of(i), nxt)
            if j % stride:
                continue
            jj = j // stride
            if jj == 0:
                qq = q_scr[i]
                qh = [qq[:, :dh], qq[:, dh:]]
            if jj < 2 * _CHUNKS:
                hh, c = divmod(jj, _CHUNKS)
                cols = slice(c * cw, (c + 1) * cw)
                s = jnp.dot(qh[hh], k_buf[i % 2, hh * dh:(hh + 1) * dh, cols],
                            preferred_element_type=_F32) * scale
                s_scr[hh, :, cols] = s
                for c2 in range(cw // 128):
                    sc = s[:, c2 * 128:(c2 + 1) * 128]
                    m[hh] = sc if m[hh] is None else jnp.maximum(m[hh], sc)
            elif jj == 2 * _CHUNKS:
                m = [jnp.max(mm, axis=-1, keepdims=True) for mm in m]
            elif jj <= 2 * _CHUNKS + 2:
                hh = jj - (2 * _CHUNKS + 1)
                p = jnp.exp(s_scr[hh] - m[hh])
                p_scr[hh] = p.astype(_BF16)
                l[hh] = jnp.sum(p, axis=-1, keepdims=True)
            elif after is not None:
                after(j)
        return l

    def pair(i, attn):
        l = v_phase(i, k_of(i + 1))
        return k_phase(i + 1, l, attn)

    last = n_pairs - 1
    attn = lax.fori_loop(0, last, pair, jnp.zeros(x.shape, _F32))

    o = [None, None]
    todo = [hh * _CHUNKS + c for c in range(_CHUNKS) for hh in range(2)]
    todo += [2 * _CHUNKS, 2 * _CHUNKS + 1]
    if _HEAD_MAJOR:
        todo = list(range(n_pv))

    def early_pv(j):
        need = (cw // 128) * (todo[0] + 1) if _HEAD_MAJOR else (nkv // _CHUNKS) * (todo[0] % _CHUNKS + 1)
        if todo[0] < 2 * _CHUNKS and j + 1 >= need:
            pv_slice(todo.pop(0), last, None, o, None)

    l = v_phase(last, mlp_blk, 2, early_pv)

    no_more = lambda b: None
    out = y = z = None
    for j in range(n3):
        _tick(j, n3 + n4, mlp_blk, no_more)
        if todo:
            attn = pv_slice(todo.pop(0), last, l, o, attn)
        elif out is None:
            hres = x + attn
            y = _layernorm(hres)
            out = hres + y
        elif z is None:
            z = _layernorm(y).astype(_BF16)

    rg = w4_buf.shape[1]
    offs = [sum(_W4_STEPS[:k]) * _R4 for k in range(len(_W4_STEPS) + 1)]
    fs = f // _W3_SLICES
    n_mxu = len(_W4_STEPS) - _VPU_STEPS
    acts, gs, gcol = [], None, None
    b = n3
    for step, n in enumerate(_W4_STEPS):
        for t in range(n):
            if step == 0 and t < _W3_SLICES:
                w = w3_buf[:, :, t * fs:(t + 1) * fs].reshape(d, fs)
                a = jnp.dot(z, w, preferred_element_type=_F32)
                acts.append(jax.nn.gelu(a, approximate=True).astype(_BF16))
            elif step == 0 and t == _W3_SLICES:
                g = jnp.concatenate(acts, axis=1)
                gs = [jnp.concatenate([g[:, k * rg + r0:k * rg + r1] for k in range(_G4)], axis=1)
                      for r0, r1 in zip(offs[:-1], offs[1:])]
                gl = jnp.concatenate(gs[n_mxu:], axis=1)
                nl = gl.shape[1]
                eye = (lax.broadcasted_iota(jnp.int32, (nl, nl), 0)
                       == lax.broadcasted_iota(jnp.int32, (nl, nl), 1))
                diag = jnp.where(eye, jnp.broadcast_to(gl[0:1].astype(_F32), (nl, nl)), 0.0)
                gcol = jnp.dot(diag.astype(_BF16), jnp.ones((nl, 128), _BF16),
                               preferred_element_type=_F32)
            _tick(b, n3 + n4, mlp_blk, no_more)
            b += 1
        r0, r1 = offs[step], offs[step + 1]
        w = w4_buf[:, r0:r1, :].reshape(_G4 * (r1 - r0), d)
        if step < n_mxu:
            out = out + jnp.dot(gs[step], w, preferred_element_type=_F32)
            if step == n_mxu - 1:
                out = jnp.where(lax.broadcasted_iota(jnp.int32, out.shape, 0) == 0, out, 0.0)
        else:
            g0 = _G4 * (r0 - offs[n_mxu])
            gc = gcol[g0:g0 + w.shape[0]]
            prod = w.astype(_F32) * jnp.concatenate([gc] * (d // 128), axis=1)
            out = out + jnp.sum(prod.reshape(w.shape[0] // _ROWS, _ROWS, d), axis=0)
    out = jnp.sum(out, axis=0, keepdims=True)
    o_ref[0] = out.astype(o_ref.dtype)


@jax.jit
def pallas_sequential_preLN__sliding_block_cached__mixer_s_mlp__decode_kernel(
    A_x: jax.Array,
    A_k_cache: jax.Array,
    A_v_cache: jax.Array,
    A_wq: jax.Array,
    A_wo: jax.Array,
    B_x: jax.Array,
    B_w1: jax.Array,
    B_w2: jax.Array,
    B_w3: jax.Array,
    B_w4: jax.Array,
):
    b, sq, d = A_x.shape
    _, n_heads, sk, dh = A_k_cache.shape
    win = min(4096, max(256, sk // 4))
    f = B_w3.shape[1]
    assert (b, sq, d, n_heads, dh, win, f) == (1, 1, 640, 32, 192, 4096, 1536)
    assert f == _G4 * _R4 * sum(_W4_STEPS)

    kt = jnp.swapaxes(A_k_cache, 2, 3).reshape(n_heads * dh, sk)
    vt = jnp.swapaxes(A_v_cache, 2, 3).reshape(n_heads * dh, sk)
    grouped = lambda w, g: w.reshape(g, w.shape[0] // g, w.shape[1])
    wq, wo = grouped(A_wq, _GQ), grouped(A_wo, _GO)
    w3, w4 = grouped(B_w3, _G3), grouped(B_w4, _G4)

    any_spec = pl.BlockSpec(memory_space=pl.ANY)
    return pl.pallas_call(
        functools.partial(_kernel, n_heads=n_heads, dh=dh, sk=sk, win=win),
        in_specs=[any_spec] * 7,
        out_specs=pl.BlockSpec(memory_space=pltpu.VMEM),
        out_shape=jax.ShapeDtypeStruct(A_x.shape, A_x.dtype),
        scratch_shapes=[
            pltpu.VMEM(A_x.shape, _BF16),
            pltpu.VMEM(wq.shape, _BF16),
            pltpu.VMEM(wo.shape, _BF16),
            pltpu.VMEM(w3.shape, _BF16),
            pltpu.VMEM(w4.shape, _BF16),
            pltpu.VMEM((2, 2 * dh, win), _BF16),
            pltpu.VMEM((2, 2 * dh, win), _BF16),
            pltpu.VMEM((n_heads // 2, _ROWS, 2 * dh), _BF16),
            pltpu.VMEM((2, _ROWS, win), _F32),
            pltpu.VMEM((2, _ROWS, win), _BF16),
            pltpu.SemaphoreType.DMA((1,)),
            pltpu.SemaphoreType.DMA((_RING,)),
        ],
        compiler_params=pltpu.CompilerParams(
            vmem_limit_bytes=64 * 1024 * 1024,
            disable_bounds_checks=True,
            disable_semaphore_checks=True,
        ),
    )(A_x, kt, vt, wq, wo, w3, w4)
```

```python
import functools

import jax
import jax.numpy as jnp
from jax import lax
import jax.experimental.pallas as pl
import jax.experimental.pallas.tpu as pltpu

_F32 = jnp.float32
_BF16 = jnp.bfloat16
_EPS = 1e-5
_ROWS = 8
_NT = (((1,), (1,)), ((), ()))

_LOOK_HI = 15
_LOOK_LO = 32
_KV_HI = 32
_STRIDE = 3
_CHUNKS = 8
_GQ, _CQ, _HQ = 10, 384, 2
_GO, _HO = 8, 3
_G3, _H3 = 4, 1
_G4, _R4, _H4 = 4, 16, 1
_W3_SLICES = 6
_W4_STEPS = (8, 8, 5, 1, 1, 1)
_VPU_STEPS = 3
_X_TICK = 24
_PRO_LO = 2
_RING = 64


def _layernorm(x):
    m = jnp.mean(x, axis=-1, keepdims=True)
    xc = x - m
    v = jnp.mean(xc * xc, axis=-1, keepdims=True)
    return xc / jnp.sqrt(v + _EPS)


def _mul(i, n, align):
    return i * n if isinstance(i, int) else pl.multiple_of(i * n, align)


class _Block:
    def __init__(self, src, dst, sem, n_hi):
        self.src, self.dst, self.sem, self.n_hi = src, dst, sem, n_hi

    def _piece(self, a, n):
        return pltpu.make_async_copy(
            self.src.at[pl.ds(a, n)], self.dst.at[pl.ds(a, n)], self.sem)

    def hi(self):
        self._piece(0, self.n_hi).start(priority=0)

    def lo(self):
        self._piece(self.n_hi, self.dst.shape[0] - self.n_hi).start(priority=1)

    def wait(self):
        pltpu.make_async_copy(self.dst, self.dst, self.sem).wait()


def _tick(j, n, cur, nxt):
    cur(j).wait()
    ahead = lambda p: cur(p) if p < n else nxt(p - n)
    bh, bl = ahead(j + _LOOK_HI), ahead(j + _LOOK_LO)
    if bh is not None:
        bh.hi()
    if bl is not None:
        bl.lo()


def _kernel(x_hbm, kt_hbm, vt_hbm, wq_hbm, wo_hbm, w3_hbm, w4_hbm, o_ref,
            x_buf, wq_buf, wo_buf, w3_buf, w4_buf, k_buf, v_buf, q_scr, s_scr, p_scr,
            x_sem, ring, *, n_heads, dh, sk, win):
    start = sk - win
    scale = dh ** -0.5
    d = x_buf.shape[-1]
    f = w3_buf.shape[-1]
    pr = 2 * dh
    n_pairs = n_heads // 2
    cw = win // _CHUNKS
    ncq = wq_buf.shape[2] // _CQ
    nq = wq_buf.shape[1] // 8 * ncq
    no = wo_buf.shape[1] // 8
    n3 = w3_buf.shape[1] // 8
    n4 = w4_buf.shape[1] // _R4
    nkv = 2 * (win // 128)
    assert nkv % _RING == 0 and nq % _RING == 0 and _LOOK_LO < _RING

    def sem(b, after_wo=True):
        return ring.at[(b + (no if after_wo else 0)) % _RING]

    def wq_blk(b):
        idx = (slice(None), pl.ds(_mul(b // ncq, 8, 8), 8), pl.ds(_mul(b % ncq, _CQ, 128), _CQ))
        return _Block(wq_hbm.at[idx], wq_buf.at[idx], sem(b, False), _HQ)

    def wo_blk(b):
        idx = (slice(None), pl.ds(_mul(b, 8, 8), 8))
        return _Block(wo_hbm.at[idx], wo_buf.at[idx], sem(b, False), _HO)

    def mlp_blk(b):
        if b < n3:
            idx = (slice(None), pl.ds(b * 8, 8))
            return _Block(w3_hbm.at[idx], w3_buf.at[idx], sem(b), _H3)
        if b < n3 + n4:
            idx = (slice(None), pl.ds((b - n3) * _R4, _R4))
            return _Block(w4_hbm.at[idx], w4_buf.at[idx], sem(b), _H4)
        return None

    def kv_stream(src, buf, i, after_wo=True):
        def blk(j):
            col, row = _mul(j % (nkv // 2), 128, 128), _mul(j // (nkv // 2), dh, 8)
            return _Block(src.at[pl.ds(_mul(i, pr, 8) + row, dh), pl.ds(start + col, 128)],
                          buf.at[i % 2, pl.ds(row, dh), pl.ds(col, 128)],
                          sem(j, after_wo), _KV_HI)
        return blk

    k_of = functools.partial(kv_stream, kt_hbm, k_buf)
    v_of = functools.partial(kv_stream, vt_hbm, v_buf)

    x_cp = pltpu.make_async_copy(x_hbm, x_buf, x_sem.at[0])
    x_cp.start()
    k0_blk = k_of(0, False)
    for b in range(_PRO_LO):
        k0_blk(b).lo()

    def first(b, c):
        k0_blk(b).hi()
        k0_blk(b + _PRO_LO).lo()
        return c
    lax.fori_loop(0, _LOOK_HI, first, 0)
    for b in range(_PRO_LO + _LOOK_HI, _LOOK_LO):
        k0_blk(b).lo()
    x = xn = None
    for j in range(nkv):
        if j == _X_TICK:
            x_cp.wait()
            x = jnp.broadcast_to(x_buf[0].astype(_F32), (_ROWS, d))
            xn = _layernorm(x).astype(_BF16)
        _tick(j, nkv, k0_blk, wq_blk)

    def wq_tick(b, c):
        wq_blk(b).wait()
        wq_blk(b + _LOOK_HI).hi()
        wq_blk(b + _LOOK_LO).lo()
        return c
    lax.fori_loop(0, nq - _LOOK_LO, wq_tick, 0)
    for j in range(nq - _LOOK_LO, nq):
        _tick(j, nq, wq_blk, wo_blk)

    per_pair = (no - _LOOK_LO) // n_pairs

    def wo_ticks(i, c):
        for t in range(per_pair):
            b = i * per_pair + t
            wo_blk(b).wait()
            wo_blk(b + _LOOK_HI).hi()
            wo_blk(b + _LOOK_LO).lo()
            if t < pr // 128:
                col = pl.multiple_of(i * pr + t * 128, 128)
                w = wq_buf[:, :, pl.ds(col, 128)].reshape(d, 128)
                q_scr[i, :, t * 128:(t + 1) * 128] = jnp.dot(
                    xn, w, preferred_element_type=_F32).astype(_BF16)
        return c
    lax.fori_loop(0, n_pairs, wo_ticks, 0)
    for j in range(per_pair * n_pairs, no):
        _tick(j, no, wo_blk, v_of(0))

    n_pv = 2 * _CHUNKS + 2

    def pv_slice(j, i, l, o, attn):
        if j < 2 * _CHUNKS:
            hh, c = divmod(j, _CHUNKS)
            cols = slice(c * cw, (c + 1) * cw)
            oj = lax.dot_general(p_scr[hh, :, cols], v_buf[i % 2, hh * dh:(hh + 1) * dh, cols],
                                 _NT, preferred_element_type=_F32)
            o[hh] = oj if o[hh] is None else oj + o[hh]
        elif j < n_pv:
            hh = j - 2 * _CHUNKS
            ppg = wo_buf.shape[1] // pr
            w = wo_buf[i // ppg, pl.ds(_mul(i % ppg, pr, 64) + hh * dh, dh), :]
            attn = attn + jnp.dot((o[hh] / l[hh]).astype(_BF16), w,
                                  preferred_element_type=_F32)
        return attn

    def k_phase(i, l, attn):
        o = [None, None]
        for j in range(nkv):
            _tick(j, nkv, k_of(i), v_of(i))
            if j % _STRIDE == 0:
                attn = pv_slice(j // _STRIDE, i - 1, l, o, attn)
        return attn

    def v_phase(i, nxt, stride=_STRIDE, after=None):
        m = [None, None]
        l = [None, None]
        qh = None
        for j in range(nkv):
            _tick(j, nkv, v_of(i), nxt)
            if j % stride:
                continue
            jj = j // stride
            if jj == 0:
                qq = q_scr[i]
                qh = [qq[:, :dh], qq[:, dh:]]
            if jj < 2 * _CHUNKS:
                hh, c = divmod(jj, _CHUNKS)
                cols = slice(c * cw, (c + 1) * cw)
                s = jnp.dot(qh[hh], k_buf[i % 2, hh * dh:(hh + 1) * dh, cols],
                            preferred_element_type=_F32) * scale
                s_scr[hh, :, cols] = s
                for c2 in range(cw // 128):
                    sc = s[:, c2 * 128:(c2 + 1) * 128]
                    m[hh] = sc if m[hh] is None else jnp.maximum(m[hh], sc)
            elif jj == 2 * _CHUNKS:
                m = [jnp.max(mm, axis=-1, keepdims=True) for mm in m]
            elif jj <= 2 * _CHUNKS + 2:
                hh = jj - (2 * _CHUNKS + 1)
                p = jnp.exp(s_scr[hh] - m[hh])
                p_scr[hh] = p.astype(_BF16)
                l[hh] = jnp.sum(p, axis=-1, keepdims=True)
            elif after is not None:
                after(j)
        return l

    def pair(i, attn):
        l = v_phase(i, k_of(i + 1))
        return k_phase(i + 1, l, attn)

    last = n_pairs - 1
    attn = lax.fori_loop(0, last, pair, jnp.zeros(x.shape, _F32))

    o = [None, None]
    todo = list(range(n_pv))

    def early_pv(j):
        if todo[0] < 2 * _CHUNKS and j + 1 >= (cw // 128) * (todo[0] + 1):
            pv_slice(todo.pop(0), last, None, o, None)

    l = v_phase(last, mlp_blk, 2, early_pv)

    no_more = lambda b: None
    out = y = z = None
    for j in range(n3):
        _tick(j, n3 + n4, mlp_blk, no_more)
        if todo:
            attn = pv_slice(todo.pop(0), last, l, o, attn)
        elif out is None:
            hres = x + attn
            y = _layernorm(hres)
            out = hres + y
        elif z is None:
            z = _layernorm(y).astype(_BF16)

    rg = w4_buf.shape[1]
    offs = [sum(_W4_STEPS[:k]) * _R4 for k in range(len(_W4_STEPS) + 1)]
    fs = f // _W3_SLICES
    n_mxu = len(_W4_STEPS) - _VPU_STEPS
    acts, gs, gcol = [], None, None
    b = n3
    for step, n in enumerate(_W4_STEPS):
        for t in range(n):
            if step == 0 and t < _W3_SLICES:
                w = w3_buf[:, :, t * fs:(t + 1) * fs].reshape(d, fs)
                a = jnp.dot(z, w, preferred_element_type=_F32)
                acts.append(jax.nn.gelu(a, approximate=True).astype(_BF16))
            elif step == 0 and t == _W3_SLICES:
                g = jnp.concatenate(acts, axis=1)
                gs = [jnp.concatenate([g[:, k * rg + r0:k * rg + r1] for k in range(_G4)], axis=1)
                      for r0, r1 in zip(offs[:-1], offs[1:])]
                gl = jnp.concatenate(gs[n_mxu:], axis=1)
                nl = gl.shape[1]
                eye = (lax.broadcasted_iota(jnp.int32, (nl, nl), 0)
                       == lax.broadcasted_iota(jnp.int32, (nl, nl), 1))
                diag = jnp.where(eye, jnp.broadcast_to(gl[0:1].astype(_F32), (nl, nl)), 0.0)
                gcol = jnp.dot(diag.astype(_BF16), jnp.ones((nl, 128), _BF16),
                               preferred_element_type=_F32)
            _tick(b, n3 + n4, mlp_blk, no_more)
            b += 1
        r0, r1 = offs[step], offs[step + 1]
        w = w4_buf[:, r0:r1, :].reshape(_G4 * (r1 - r0), d)
        if step < n_mxu:
            out = out + jnp.dot(gs[step], w, preferred_element_type=_F32)
            if step == n_mxu - 1:
                out = jnp.where(lax.broadcasted_iota(jnp.int32, out.shape, 0) == 0, out, 0.0)
        else:
            g0 = _G4 * (r0 - offs[n_mxu])
            gc = gcol[g0:g0 + w.shape[0]]
            prod = w.astype(_F32) * jnp.concatenate([gc] * (d // 128), axis=1)
            out = out + jnp.sum(prod.reshape(w.shape[0] // _ROWS, _ROWS, d), axis=0)
    out = jnp.sum(out, axis=0, keepdims=True)
    o_ref[0] = out.astype(o_ref.dtype)


@jax.jit
def pallas_sequential_preLN__sliding_block_cached__mixer_s_mlp__decode_kernel(
    A_x: jax.Array,
    A_k_cache: jax.Array,
    A_v_cache: jax.Array,
    A_wq: jax.Array,
    A_wo: jax.Array,
    B_x: jax.Array,
    B_w1: jax.Array,
    B_w2: jax.Array,
    B_w3: jax.Array,
    B_w4: jax.Array,
):
    b, sq, d = A_x.shape
    _, n_heads, sk, dh = A_k_cache.shape
    win = min(4096, max(256, sk // 4))
    f = B_w3.shape[1]
    assert (b, sq, d, n_heads, dh, win, f) == (1, 1, 640, 32, 192, 4096, 1536)
    assert f == _G4 * _R4 * sum(_W4_STEPS)

    kt = jnp.swapaxes(A_k_cache, 2, 3).reshape(n_heads * dh, sk)
    vt = jnp.swapaxes(A_v_cache, 2, 3).reshape(n_heads * dh, sk)
    grouped = lambda w, g: w.reshape(g, w.shape[0] // g, w.shape[1])
    wq, wo = grouped(A_wq, _GQ), grouped(A_wo, _GO)
    w3, w4 = grouped(B_w3, _G3), grouped(B_w4, _G4)

    any_spec = pl.BlockSpec(memory_space=pl.ANY)
    return pl.pallas_call(
        functools.partial(_kernel, n_heads=n_heads, dh=dh, sk=sk, win=win),
        in_specs=[any_spec] * 7,
        out_specs=pl.BlockSpec(memory_space=pltpu.VMEM),
        out_shape=jax.ShapeDtypeStruct(A_x.shape, A_x.dtype),
        scratch_shapes=[
            pltpu.VMEM(A_x.shape, _BF16),
            pltpu.VMEM(wq.shape, _BF16),
            pltpu.VMEM(wo.shape, _BF16),
            pltpu.VMEM(w3.shape, _BF16),
            pltpu.VMEM(w4.shape, _BF16),
            pltpu.VMEM((2, 2 * dh, win), _BF16),
            pltpu.VMEM((2, 2 * dh, win), _BF16),
            pltpu.VMEM((n_heads // 2, _ROWS, 2 * dh), _BF16),
            pltpu.VMEM((2, _ROWS, win), _F32),
            pltpu.VMEM((2, _ROWS, win), _BF16),
            pltpu.SemaphoreType.DMA((1,)),
            pltpu.SemaphoreType.DMA((_RING,)),
        ],
        compiler_params=pltpu.CompilerParams(
            vmem_limit_bytes=64 * 1024 * 1024,
            disable_bounds_checks=True,
            disable_semaphore_checks=True,
        ),
    )(A_x, kt, vt, wq, wo, w3, w4)
```

```python
import functools

import jax
import jax.numpy as jnp
from jax import lax
import jax.experimental.pallas as pl
import jax.experimental.pallas.tpu as pltpu

_F32 = jnp.float32
_BF16 = jnp.bfloat16
_EPS = 1e-5
_ROWS = 8
_NT = (((1,), (1,)), ((), ()))

_LOOK_HI = 15
_LOOK_LO = 32
_KV_HI = 32
_STRIDE = 3
_CHUNKS = 8
_GQ, _CQ, _HQ = 10, 384, 2
_GO, _HO = 8, 3
_G3, _H3 = 4, 1
_G4, _R4, _H4 = 4, 16, 1
_W3_SLICES = 6
_W4_STEPS = (8, 8, 5, 1, 1, 1)
_VPU_STEPS = 3
_X_TICK = 24
_PRO_LO = 2
_RING = 64


def _layernorm(x):
    m = jnp.mean(x, axis=-1, keepdims=True)
    xc = x - m
    v = jnp.mean(xc * xc, axis=-1, keepdims=True)
    return xc / jnp.sqrt(v + _EPS)


def _mul(i, n, align):
    return i * n if isinstance(i, int) else pl.multiple_of(i * n, align)


class _Block:
    def __init__(self, src, dst, sem, n_hi):
        self.src, self.dst, self.sem, self.n_hi = src, dst, sem, n_hi

    def _piece(self, a, n):
        return pltpu.make_async_copy(
            self.src.at[pl.ds(a, n)], self.dst.at[pl.ds(a, n)], self.sem)

    def hi(self):
        self._piece(0, self.n_hi).start(priority=0)

    def lo(self):
        self._piece(self.n_hi, self.dst.shape[0] - self.n_hi).start(priority=1)

    def wait(self):
        pltpu.make_async_copy(self.dst, self.dst, self.sem).wait()


def _tick(j, n, cur, nxt):
    cur(j).wait()
    ahead = lambda p: cur(p) if p < n else nxt(p - n)
    bh, bl = ahead(j + _LOOK_HI), ahead(j + _LOOK_LO)
    if bh is not None:
        bh.hi()
    if bl is not None:
        bl.lo()


def _body(x_hbm, kt_hbm, vt_hbm, wq_hbm, wo_hbm, w3_hbm, w4_hbm, o_ref,
          x_buf, wq_buf, wo_buf, w3_buf, w4_buf, k_buf, v_buf, q_scr, s_scr, p_scr,
          x_sem, ring, *, n_heads, dh, sk, win):
    start = sk - win
    scale = dh ** -0.5
    d = x_buf.shape[-1]
    f = w3_buf.shape[-1]
    pr = 2 * dh
    n_pairs = n_heads // 2
    cw = win // _CHUNKS
    ncq = wq_buf.shape[2] // _CQ
    nq = wq_buf.shape[1] // 8 * ncq
    no = wo_buf.shape[1] // 8
    n3 = w3_buf.shape[1] // 8
    n4 = w4_buf.shape[1] // _R4
    nkv = 2 * (win // 128)
    assert nkv % _RING == 0 and nq % _RING == 0 and _LOOK_LO < _RING

    def sem(b, after_wo=True):
        return ring.at[(b + (no if after_wo else 0)) % _RING]

    def wq_blk(b):
        idx = (slice(None), pl.ds(_mul(b // ncq, 8, 8), 8), pl.ds(_mul(b % ncq, _CQ, 128), _CQ))
        return _Block(wq_hbm.at[idx], wq_buf.at[idx], sem(b, False), _HQ)

    def wo_blk(b):
        idx = (slice(None), pl.ds(_mul(b, 8, 8), 8))
        return _Block(wo_hbm.at[idx], wo_buf.at[idx], sem(b, False), _HO)

    def mlp_blk(b):
        if b < n3:
            idx = (slice(None), pl.ds(b * 8, 8))
            return _Block(w3_hbm.at[idx], w3_buf.at[idx], sem(b), _H3)
        if b < n3 + n4:
            idx = (slice(None), pl.ds((b - n3) * _R4, _R4))
            return _Block(w4_hbm.at[idx], w4_buf.at[idx], sem(b), _H4)
        return None

    def kv_stream(src, buf, i, after_wo=True):
        def blk(j):
            col, row = _mul(j % (nkv // 2), 128, 128), _mul(j // (nkv // 2), dh, 8)
            return _Block(src.at[pl.ds(_mul(i, pr, 8) + row, dh), pl.ds(start + col, 128)],
                          buf.at[i % 2, pl.ds(row, dh), pl.ds(col, 128)],
                          sem(j, after_wo), _KV_HI)
        return blk

    k_of = functools.partial(kv_stream, kt_hbm, k_buf)
    v_of = functools.partial(kv_stream, vt_hbm, v_buf)

    x_cp = pltpu.make_async_copy(x_hbm, x_buf, x_sem.at[0])
    x_cp.start()
    k0_blk = k_of(0, False)
    for b in range(_PRO_LO):
        k0_blk(b).lo()

    def first(b, c):
        k0_blk(b).hi()
        k0_blk(b + _PRO_LO).lo()
        return c
    lax.fori_loop(0, _LOOK_HI, first, 0)
    for b in range(_PRO_LO + _LOOK_HI, _LOOK_LO):
        k0_blk(b).lo()
    x = xn = None
    for j in range(nkv):
        if j == _X_TICK:
            x_cp.wait()
            x = jnp.broadcast_to(x_buf[0].astype(_F32), (_ROWS, d))
            xn = _layernorm(x).astype(_BF16)
        _tick(j, nkv, k0_blk, wq_blk)

    def wq_tick(b, c):
        wq_blk(b).wait()
        wq_blk(b + _LOOK_HI).hi()
        wq_blk(b + _LOOK_LO).lo()
        return c
    lax.fori_loop(0, nq - _LOOK_LO, wq_tick, 0)
    for j in range(nq - _LOOK_LO, nq):
        _tick(j, nq, wq_blk, wo_blk)

    per_pair = (no - _LOOK_LO) // n_pairs

    def wo_ticks(i, c):
        for t in range(per_pair):
            b = i * per_pair + t
            wo_blk(b).wait()
            wo_blk(b + _LOOK_HI).hi()
            wo_blk(b + _LOOK_LO).lo()
            if t < pr // 128:
                col = pl.multiple_of(i * pr + t * 128, 128)
                w = wq_buf[:, :, pl.ds(col, 128)].reshape(d, 128)
                q_scr[i, :, t * 128:(t + 1) * 128] = jnp.dot(
                    xn, w, preferred_element_type=_F32).astype(_BF16)
        return c
    lax.fori_loop(0, n_pairs, wo_ticks, 0)
    for j in range(per_pair * n_pairs, no):
        _tick(j, no, wo_blk, v_of(0))

    n_pv = 2 * _CHUNKS + 2

    def pv_slice(j, i, l, o, attn):
        if j < 2 * _CHUNKS:
            hh, c = divmod(j, _CHUNKS)
            cols = slice(c * cw, (c + 1) * cw)
            oj = lax.dot_general(p_scr[hh, :, cols], v_buf[i % 2, hh * dh:(hh + 1) * dh, cols],
                                 _NT, preferred_element_type=_F32)
            o[hh] = oj if o[hh] is None else oj + o[hh]
        elif j < n_pv:
            hh = j - 2 * _CHUNKS
            ppg = wo_buf.shape[1] // pr
            w = wo_buf[i // ppg, pl.ds(_mul(i % ppg, pr, 64) + hh * dh, dh), :]
            attn = attn + jnp.dot((o[hh] / l[hh]).astype(_BF16), w,
                                  preferred_element_type=_F32)
        return attn

    def k_phase(i, l, attn):
        o = [None, None]
        for j in range(nkv):
            _tick(j, nkv, k_of(i), v_of(i))
            if j % _STRIDE == 0:
                attn = pv_slice(j // _STRIDE, i - 1, l, o, attn)
        return attn

    def v_phase(i, nxt, stride=_STRIDE, after=None):
        m = [None, None]
        l = [None, None]
        qh = None
        for j in range(nkv):
            _tick(j, nkv, v_of(i), nxt)
            if j % stride:
                continue
            jj = j // stride
            if jj == 0:
                qq = q_scr[i]
                qh = [qq[:, :dh], qq[:, dh:]]
            if jj < 2 * _CHUNKS:
                hh, c = divmod(jj, _CHUNKS)
                cols = slice(c * cw, (c + 1) * cw)
                s = jnp.dot(qh[hh], k_buf[i % 2, hh * dh:(hh + 1) * dh, cols],
                            preferred_element_type=_F32) * scale
                s_scr[hh, :, cols] = s
                for c2 in range(cw // 128):
                    sc = s[:, c2 * 128:(c2 + 1) * 128]
                    m[hh] = sc if m[hh] is None else jnp.maximum(m[hh], sc)
            elif jj == 2 * _CHUNKS:
                m = [jnp.max(mm, axis=-1, keepdims=True) for mm in m]
            elif jj <= 2 * _CHUNKS + 2:
                hh = jj - (2 * _CHUNKS + 1)
                p = jnp.exp(s_scr[hh] - m[hh])
                p_scr[hh] = p.astype(_BF16)
                l[hh] = jnp.sum(p, axis=-1, keepdims=True)
            elif after is not None:
                after(j)
        return l

    def pair(i, attn):
        l = v_phase(i, k_of(i + 1))
        return k_phase(i + 1, l, attn)

    last = n_pairs - 1
    attn = lax.fori_loop(0, last, pair, jnp.zeros(x.shape, _F32))

    o = [None, None]
    todo = list(range(n_pv))

    def early_pv(j):
        if todo[0] < 2 * _CHUNKS and j + 1 >= (cw // 128) * (todo[0] + 1):
            pv_slice(todo.pop(0), last, None, o, None)

    l = v_phase(last, mlp_blk, 2, early_pv)

    no_more = lambda b: None
    out = y = z = None
    for j in range(n3):
        _tick(j, n3 + n4, mlp_blk, no_more)
        if todo:
            attn = pv_slice(todo.pop(0), last, l, o, attn)
        elif out is None:
            hres = x + attn
            y = _layernorm(hres)
            out = hres + y
        elif z is None:
            z = _layernorm(y).astype(_BF16)

    rg = w4_buf.shape[1]
    offs = [sum(_W4_STEPS[:k]) * _R4 for k in range(len(_W4_STEPS) + 1)]
    fs = f // _W3_SLICES
    n_mxu = len(_W4_STEPS) - _VPU_STEPS
    acts, gs, gcol = [], None, None
    b = n3
    for step, n in enumerate(_W4_STEPS):
        for t in range(n):
            if step == 0 and t < _W3_SLICES:
                w = w3_buf[:, :, t * fs:(t + 1) * fs].reshape(d, fs)
                a = jnp.dot(z, w, preferred_element_type=_F32)
                acts.append(jax.nn.gelu(a, approximate=True).astype(_BF16))
            elif step == 0 and t == _W3_SLICES:
                g = jnp.concatenate(acts, axis=1)
                gs = [jnp.concatenate([g[:, k * rg + r0:k * rg + r1] for k in range(_G4)], axis=1)
                      for r0, r1 in zip(offs[:-1], offs[1:])]
                gl = jnp.concatenate(gs[n_mxu:], axis=1)
                nl = gl.shape[1]
                eye = (lax.broadcasted_iota(jnp.int32, (nl, nl), 0)
                       == lax.broadcasted_iota(jnp.int32, (nl, nl), 1))
                diag = jnp.where(eye, jnp.broadcast_to(gl[0:1].astype(_F32), (nl, nl)), 0.0)
                gcol = jnp.dot(diag.astype(_BF16), jnp.ones((nl, 128), _BF16),
                               preferred_element_type=_F32)
            _tick(b, n3 + n4, mlp_blk, no_more)
            b += 1
        r0, r1 = offs[step], offs[step + 1]
        w = w4_buf[:, r0:r1, :].reshape(_G4 * (r1 - r0), d)
        if step < n_mxu:
            out = out + jnp.dot(gs[step], w, preferred_element_type=_F32)
            if step == n_mxu - 1:
                out = jnp.where(lax.broadcasted_iota(jnp.int32, out.shape, 0) == 0, out, 0.0)
        else:
            g0 = _G4 * (r0 - offs[n_mxu])
            gc = gcol[g0:g0 + w.shape[0]]
            prod = w.astype(_F32) * jnp.concatenate([gc] * (d // 128), axis=1)
            out = out + jnp.sum(prod.reshape(w.shape[0] // _ROWS, _ROWS, d), axis=0)
    out = jnp.sum(out, axis=0, keepdims=True)
    o_ref[0] = out.astype(o_ref.dtype)


def _kernel(*refs, **static):
    pl.run_scoped(functools.partial(_body, *refs, **static),
                  pltpu.SemaphoreType.DMA((1,)), pltpu.SemaphoreType.DMA((_RING,)))


@jax.jit
def pallas_sequential_preLN__sliding_block_cached__mixer_s_mlp__decode_kernel(
    A_x: jax.Array,
    A_k_cache: jax.Array,
    A_v_cache: jax.Array,
    A_wq: jax.Array,
    A_wo: jax.Array,
    B_x: jax.Array,
    B_w1: jax.Array,
    B_w2: jax.Array,
    B_w3: jax.Array,
    B_w4: jax.Array,
):
    b, sq, d = A_x.shape
    _, n_heads, sk, dh = A_k_cache.shape
    win = min(4096, max(256, sk // 4))
    f = B_w3.shape[1]
    assert (b, sq, d, n_heads, dh, win, f) == (1, 1, 640, 32, 192, 4096, 1536)
    assert f == _G4 * _R4 * sum(_W4_STEPS)

    kt = jnp.swapaxes(A_k_cache, 2, 3).reshape(n_heads * dh, sk)
    vt = jnp.swapaxes(A_v_cache, 2, 3).reshape(n_heads * dh, sk)
    grouped = lambda w, g: w.reshape(g, w.shape[0] // g, w.shape[1])
    wq, wo = grouped(A_wq, _GQ), grouped(A_wo, _GO)
    w3, w4 = grouped(B_w3, _G3), grouped(B_w4, _G4)

    any_spec = pl.BlockSpec(memory_space=pl.ANY)
    return pl.pallas_call(
        functools.partial(_kernel, n_heads=n_heads, dh=dh, sk=sk, win=win),
        in_specs=[any_spec] * 7,
        out_specs=pl.BlockSpec(memory_space=pltpu.VMEM),
        out_shape=jax.ShapeDtypeStruct(A_x.shape, A_x.dtype),
        scratch_shapes=[
            pltpu.VMEM(A_x.shape, _BF16),
            pltpu.VMEM(wq.shape, _BF16),
            pltpu.VMEM(wo.shape, _BF16),
            pltpu.VMEM(w3.shape, _BF16),
            pltpu.VMEM(w4.shape, _BF16),
            pltpu.VMEM((2, 2 * dh, win), _BF16),
            pltpu.VMEM((2, 2 * dh, win), _BF16),
            pltpu.VMEM((n_heads // 2, _ROWS, 2 * dh), _BF16),
            pltpu.VMEM((2, _ROWS, win), _F32),
            pltpu.VMEM((2, _ROWS, win), _BF16),
        ],
        compiler_params=pltpu.CompilerParams(vmem_limit_bytes=64 * 1024 * 1024),
    )(A_x, kt, vt, wq, wo, w3, w4)
```

```python
import functools

import jax
import jax.numpy as jnp
from jax import lax
import jax.experimental.pallas as pl
import jax.experimental.pallas.tpu as pltpu

_F32 = jnp.float32
_BF16 = jnp.bfloat16
_EPS = 1e-5
_ROWS = 8
_NT = (((1,), (1,)), ((), ()))

_LOOK_HI = 15
_LOOK_LO = 32
_KV_HI = 32
_STRIDE = 3
_CHUNKS = 8
_GQ, _CQ, _HQ = 10, 384, 2
_GO, _HO = 8, 3
_G3, _H3 = 4, 1
_G4, _R4, _H4 = 4, 16, 1
_W3_SLICES = 6
_W4_STEPS = (8, 8, 5, 1, 1, 1)
_VPU_STEPS = 3
_X_TICK = 24
_PRO_LO = 2
_RING = 64


def _layernorm(x):
    m = jnp.mean(x, axis=-1, keepdims=True)
    xc = x - m
    v = jnp.mean(xc * xc, axis=-1, keepdims=True)
    return xc / jnp.sqrt(v + _EPS)


def _mul(i, n, align):
    return i * n if isinstance(i, int) else pl.multiple_of(i * n, align)


class _Block:
    def __init__(self, src, dst, sem, n_hi):
        self.src, self.dst, self.sem, self.n_hi = src, dst, sem, n_hi

    def _piece(self, a, n):
        return pltpu.make_async_copy(
            self.src.at[pl.ds(a, n)], self.dst.at[pl.ds(a, n)], self.sem)

    def hi(self):
        self._piece(0, self.n_hi).start(priority=0)

    def lo(self):
        self._piece(self.n_hi, self.dst.shape[0] - self.n_hi).start(priority=1)

    def wait(self):
        pltpu.make_async_copy(self.dst, self.dst, self.sem).wait()


def _tick(j, n, cur, nxt):
    cur(j).wait()
    ahead = lambda p: cur(p) if p < n else nxt(p - n)
    bh, bl = ahead(j + _LOOK_HI), ahead(j + _LOOK_LO)
    if bh is not None:
        bh.hi()
    if bl is not None:
        bl.lo()


def _body(x_hbm, kt_hbm, vt_hbm, wq_hbm, wo_hbm, w3_hbm, w4_hbm, o_ref,
          x_buf, wq_buf, wo_buf, w3_buf, w4_buf, k_buf, v_buf, q_scr, s_scr, p_scr,
          x_sem, ring, *, n_heads, dh, sk, win):
    start = sk - win
    scale = dh ** -0.5
    d = x_buf.shape[-1]
    f = w3_buf.shape[-1]
    pr = 2 * dh
    n_pairs = n_heads // 2
    cw = win // _CHUNKS
    ncq = wq_buf.shape[2] // _CQ
    nq = wq_buf.shape[1] // 8 * ncq
    no = wo_buf.shape[1] // 8
    n3 = w3_buf.shape[1] // 8
    n4 = w4_buf.shape[1] // _R4
    nkv = 2 * (win // 128)
    assert nkv % _RING == 0 and nq % _RING == 0 and _LOOK_LO < _RING

    def sem(b, after_wo=True):
        return ring.at[(b + (no if after_wo else 0)) % _RING]

    def wq_blk(b, r=0):
        idx = (slice(None), pl.ds(_mul(r + b // ncq, 8, 8), 8), pl.ds(b % ncq * _CQ, _CQ))
        return _Block(wq_hbm.at[idx], wq_buf.at[idx], sem(r * ncq + b, False), _HQ)

    def wo_blk(b):
        idx = (slice(None), pl.ds(_mul(b, 8, 8), 8))
        return _Block(wo_hbm.at[idx], wo_buf.at[idx], sem(b, False), _HO)

    def mlp_blk(b):
        if b < n3:
            idx = (slice(None), pl.ds(b * 8, 8))
            return _Block(w3_hbm.at[idx], w3_buf.at[idx], sem(b), _H3)
        if b < n3 + n4:
            idx = (slice(None), pl.ds((b - n3) * _R4, _R4))
            return _Block(w4_hbm.at[idx], w4_buf.at[idx], sem(b), _H4)
        return None

    def kv_stream(src, buf, i, after_wo=True):
        def blk(j):
            col, row = _mul(j % (nkv // 2), 128, 128), _mul(j // (nkv // 2), dh, 8)
            return _Block(src.at[pl.ds(_mul(i, pr, 8) + row, dh), pl.ds(start + col, 128)],
                          buf.at[i % 2, pl.ds(row, dh), pl.ds(col, 128)],
                          sem(j, after_wo), _KV_HI)
        return blk

    k_of = functools.partial(kv_stream, kt_hbm, k_buf)
    v_of = functools.partial(kv_stream, vt_hbm, v_buf)

    x_cp = pltpu.make_async_copy(x_hbm, x_buf, x_sem.at[0])
    x_cp.start()
    k0_blk = k_of(0, False)
    for b in range(_PRO_LO):
        k0_blk(b).lo()

    def first(b, c):
        k0_blk(b).hi()
        k0_blk(b + _PRO_LO).lo()
        return c
    lax.fori_loop(0, _LOOK_HI, first, 0)
    for b in range(_PRO_LO + _LOOK_HI, _LOOK_LO):
        k0_blk(b).lo()
    x = xn = None
    for j in range(nkv):
        if j == _X_TICK:
            x_cp.wait()
            x = jnp.broadcast_to(x_buf[0].astype(_F32), (_ROWS, d))
            xn = _layernorm(x).astype(_BF16)
        _tick(j, nkv, k0_blk, wq_blk)

    def wq_ticks(r, c):
        for b in range(ncq):
            wq_blk(b, r).wait()
            wq_blk(b + _LOOK_HI, r).hi()
            wq_blk(b + _LOOK_LO, r).lo()
        return c
    n_rolled = (nq - _LOOK_LO) // ncq
    lax.fori_loop(0, n_rolled, wq_ticks, 0)
    for j in range(n_rolled * ncq, nq):
        _tick(j, nq, wq_blk, wo_blk)

    per_pair = (no - _LOOK_LO) // n_pairs

    def wo_ticks(i, c):
        for t in range(per_pair):
            b = i * per_pair + t
            wo_blk(b).wait()
            wo_blk(b + _LOOK_HI).hi()
            wo_blk(b + _LOOK_LO).lo()
            if t < pr // 128:
                col = pl.multiple_of(i * pr + t * 128, 128)
                w = wq_buf[:, :, pl.ds(col, 128)].reshape(d, 128)
                q_scr[i, :, t * 128:(t + 1) * 128] = jnp.dot(
                    xn, w, preferred_element_type=_F32).astype(_BF16)
        return c
    lax.fori_loop(0, n_pairs, wo_ticks, 0)
    for j in range(per_pair * n_pairs, no):
        _tick(j, no, wo_blk, v_of(0))

    n_pv = 2 * _CHUNKS + 2

    def pv_slice(j, i, l, o, attn):
        if j < 2 * _CHUNKS:
            hh, c = divmod(j, _CHUNKS)
            cols = slice(c * cw, (c + 1) * cw)
            oj = lax.dot_general(p_scr[hh, :, cols], v_buf[i % 2, hh * dh:(hh + 1) * dh, cols],
                                 _NT, preferred_element_type=_F32)
            o[hh] = oj if o[hh] is None else oj + o[hh]
        elif j < n_pv:
            hh = j - 2 * _CHUNKS
            ppg = wo_buf.shape[1] // pr
            w = wo_buf[i // ppg, pl.ds(_mul(i % ppg, pr, 64) + hh * dh, dh), :]
            attn = attn + jnp.dot((o[hh] / l[hh]).astype(_BF16), w,
                                  preferred_element_type=_F32)
        return attn

    def k_phase(i, l, attn):
        o = [None, None]
        for j in range(nkv):
            _tick(j, nkv, k_of(i), v_of(i))
            if j % _STRIDE == 0:
                attn = pv_slice(j // _STRIDE, i - 1, l, o, attn)
        return attn

    def v_phase(i, nxt, stride=_STRIDE, after=None):
        m = [None, None]
        l = [None, None]
        qh = None
        for j in range(nkv):
            _tick(j, nkv, v_of(i), nxt)
            if j % stride:
                continue
            jj = j // stride
            if jj == 0:
                qq = q_scr[i]
                qh = [qq[:, :dh], qq[:, dh:]]
            if jj < 2 * _CHUNKS:
                hh, c = divmod(jj, _CHUNKS)
                cols = slice(c * cw, (c + 1) * cw)
                s = jnp.dot(qh[hh], k_buf[i % 2, hh * dh:(hh + 1) * dh, cols],
                            preferred_element_type=_F32) * scale
                s_scr[hh, :, cols] = s
                for c2 in range(cw // 128):
                    sc = s[:, c2 * 128:(c2 + 1) * 128]
                    m[hh] = sc if m[hh] is None else jnp.maximum(m[hh], sc)
            elif jj == 2 * _CHUNKS:
                m = [jnp.max(mm, axis=-1, keepdims=True) for mm in m]
            elif jj <= 2 * _CHUNKS + 2:
                hh = jj - (2 * _CHUNKS + 1)
                p = jnp.exp(s_scr[hh] - m[hh])
                p_scr[hh] = p.astype(_BF16)
                l[hh] = jnp.sum(p, axis=-1, keepdims=True)
            elif after is not None:
                after(j)
        return l

    def pair(i, attn):
        l = v_phase(i, k_of(i + 1))
        return k_phase(i + 1, l, attn)

    last = n_pairs - 1
    attn = lax.fori_loop(0, last, pair, jnp.zeros(x.shape, _F32))

    o = [None, None]
    todo = list(range(n_pv))

    def early_pv(j):
        if todo[0] < 2 * _CHUNKS and j + 1 >= (cw // 128) * (todo[0] + 1):
            pv_slice(todo.pop(0), last, None, o, None)

    l = v_phase(last, mlp_blk, 2, early_pv)

    no_more = lambda b: None
    out = y = z = None
    for j in range(n3):
        _tick(j, n3 + n4, mlp_blk, no_more)
        if todo:
            attn = pv_slice(todo.pop(0), last, l, o, attn)
        elif out is None:
            hres = x + attn
            y = _layernorm(hres)
            out = hres + y
        elif z is None:
            z = _layernorm(y).astype(_BF16)

    rg = w4_buf.shape[1]
    offs = [sum(_W4_STEPS[:k]) * _R4 for k in range(len(_W4_STEPS) + 1)]
    fs = f // _W3_SLICES
    n_mxu = len(_W4_STEPS) - _VPU_STEPS
    acts, gs, gcol = [], None, None
    b = n3
    for step, n in enumerate(_W4_STEPS):
        for t in range(n):
            if step == 0 and t < _W3_SLICES:
                w = w3_buf[:, :, t * fs:(t + 1) * fs].reshape(d, fs)
                a = jnp.dot(z, w, preferred_element_type=_F32)
                acts.append(jax.nn.gelu(a, approximate=True).astype(_BF16))
            elif step == 0 and t == _W3_SLICES:
                g = jnp.concatenate(acts, axis=1)
                gs = [jnp.concatenate([g[:, k * rg + r0:k * rg + r1] for k in range(_G4)], axis=1)
                      for r0, r1 in zip(offs[:-1], offs[1:])]
                gl = jnp.concatenate(gs[n_mxu:], axis=1)
                nl = gl.shape[1]
                eye = (lax.broadcasted_iota(jnp.int32, (nl, nl), 0)
                       == lax.broadcasted_iota(jnp.int32, (nl, nl), 1))
                diag = jnp.where(eye, jnp.broadcast_to(gl[0:1].astype(_F32), (nl, nl)), 0.0)
                gcol = jnp.dot(diag.astype(_BF16), jnp.ones((nl, 128), _BF16),
                               preferred_element_type=_F32)
            _tick(b, n3 + n4, mlp_blk, no_more)
            b += 1
        r0, r1 = offs[step], offs[step + 1]
        w = w4_buf[:, r0:r1, :].reshape(_G4 * (r1 - r0), d)
        if step < n_mxu:
            out = out + jnp.dot(gs[step], w, preferred_element_type=_F32)
            if step == n_mxu - 1:
                out = jnp.where(lax.broadcasted_iota(jnp.int32, out.shape, 0) == 0, out, 0.0)
        else:
            g0 = _G4 * (r0 - offs[n_mxu])
            gc = gcol[g0:g0 + w.shape[0]]
            prod = w.astype(_F32) * jnp.concatenate([gc] * (d // 128), axis=1)
            out = out + jnp.sum(prod.reshape(w.shape[0] // _ROWS, _ROWS, d), axis=0)
    out = jnp.sum(out, axis=0, keepdims=True)
    o_ref[0] = out.astype(o_ref.dtype)


def _kernel(*refs, **static):
    pl.run_scoped(functools.partial(_body, *refs, **static),
                  pltpu.SemaphoreType.DMA((1,)), pltpu.SemaphoreType.DMA((_RING,)))


@jax.jit
def pallas_sequential_preLN__sliding_block_cached__mixer_s_mlp__decode_kernel(
    A_x: jax.Array,
    A_k_cache: jax.Array,
    A_v_cache: jax.Array,
    A_wq: jax.Array,
    A_wo: jax.Array,
    B_x: jax.Array,
    B_w1: jax.Array,
    B_w2: jax.Array,
    B_w3: jax.Array,
    B_w4: jax.Array,
):
    b, sq, d = A_x.shape
    _, n_heads, sk, dh = A_k_cache.shape
    win = min(4096, max(256, sk // 4))
    f = B_w3.shape[1]
    assert (b, sq, d, n_heads, dh, win, f) == (1, 1, 640, 32, 192, 4096, 1536)
    assert f == _G4 * _R4 * sum(_W4_STEPS)

    kt = jnp.swapaxes(A_k_cache, 2, 3).reshape(n_heads * dh, sk)
    vt = jnp.swapaxes(A_v_cache, 2, 3).reshape(n_heads * dh, sk)
    grouped = lambda w, g: w.reshape(g, w.shape[0] // g, w.shape[1])
    wq, wo = grouped(A_wq, _GQ), grouped(A_wo, _GO)
    w3, w4 = grouped(B_w3, _G3), grouped(B_w4, _G4)

    any_spec = pl.BlockSpec(memory_space=pl.ANY)
    return pl.pallas_call(
        functools.partial(_kernel, n_heads=n_heads, dh=dh, sk=sk, win=win),
        in_specs=[any_spec] * 7,
        out_specs=pl.BlockSpec(memory_space=pltpu.VMEM),
        out_shape=jax.ShapeDtypeStruct(A_x.shape, A_x.dtype),
        scratch_shapes=[
            pltpu.VMEM(A_x.shape, _BF16),
            pltpu.VMEM(wq.shape, _BF16),
            pltpu.VMEM(wo.shape, _BF16),
            pltpu.VMEM(w3.shape, _BF16),
            pltpu.VMEM(w4.shape, _BF16),
            pltpu.VMEM((2, 2 * dh, win), _BF16),
            pltpu.VMEM((2, 2 * dh, win), _BF16),
            pltpu.VMEM((n_heads // 2, _ROWS, 2 * dh), _BF16),
            pltpu.VMEM((2, _ROWS, win), _F32),
            pltpu.VMEM((2, _ROWS, win), _BF16),
        ],
        compiler_params=pltpu.CompilerParams(vmem_limit_bytes=64 * 1024 * 1024),
    )(A_x, kt, vt, wq, wo, w3, w4)
```

```python
import functools

import jax
import jax.numpy as jnp
from jax import lax
import jax.experimental.pallas as pl
import jax.experimental.pallas.tpu as pltpu

_F32 = jnp.float32
_BF16 = jnp.bfloat16
_EPS = 1e-5
_ROWS = 8
_NT = (((1,), (1,)), ((), ()))

_LOOK_HI = 15
_LOOK_LO = 28
_PRO_LO = 2
_RING = 64
_KV_HI = 32
_STRIDE = 3
_CHUNKS = 8
_GT = 256
_G3, _G4, _R4 = 4, 4, 16
_W3_SLICES = 6
_W4_STEPS = (8, 8, 5, 1, 1, 1)
_VPU_STEPS = 3


def _layernorm(x):
    m = jnp.mean(x, axis=-1, keepdims=True)
    xc = x - m
    v = jnp.mean(xc * xc, axis=-1, keepdims=True)
    return xc / jnp.sqrt(v + _EPS)


def _mul(i, n, align):
    return i * n if isinstance(i, int) else pl.multiple_of(i * n, align)


def _divmod2(i, n):
    if isinstance(i, int):
        return divmod(i, n)
    return lax.shift_right_logical(i, n.bit_length() - 1), lax.bitwise_and(i, n - 1)


class _Block:
    def __init__(self, src, dst, sem, n_hi, extra=None):
        self.src, self.dst, self.sem, self.n_hi, self.extra = src, dst, sem, n_hi, extra

    def _piece(self, a, n):
        return pltpu.make_async_copy(
            self.src.at[pl.ds(a, n)], self.dst.at[pl.ds(a, n)], self.sem)

    def hi(self):
        self._piece(0, self.n_hi).start(priority=0)

    def lo(self):
        self._piece(self.n_hi, self.dst.shape[0] - self.n_hi).start(priority=1)
        if self.extra is not None:
            pltpu.make_async_copy(*self.extra).start(priority=1)

    def wait(self):
        pltpu.make_async_copy(self.dst, self.dst, self.sem).wait()
        if self.extra is not None:
            pltpu.make_async_copy(*self.extra).wait()


def _tick(j, n, cur, nxt):
    cur(j).wait()
    ahead = lambda p: cur(p) if p < n else nxt(p - n)
    bh, bl = ahead(j + _LOOK_HI), ahead(j + _LOOK_LO)
    if bh is not None:
        bh.hi()
    if bl is not None:
        bl.lo()


def _body(x_hbm, kt_hbm, vt_hbm, wq_hbm, wo_hbm, w3_hbm, w4_hbm, o_ref,
          x_buf, wq_buf, wo_buf, w3_buf, w4_buf, k_buf, v_buf, q_scr, s_scr, p_scr,
          x_sem, ring, ring2, *, n_heads, dh, sk, win):
    start = sk - win
    scale = dh ** -0.5
    d = x_buf.shape[-1]
    f = w3_buf.shape[-1]
    pr = 2 * dh
    n_pairs = n_heads // 2
    cw = win // _CHUNKS
    n3 = w3_buf.shape[1] // 8
    n4 = w4_buf.shape[1] // _R4
    nkv = 2 * (win // 128)
    assert nkv % _RING == 0 and _GT % _RING == 0 and _LOOK_LO < _RING

    def w_blk(b):
        r = pl.ds(_mul(b, 8, 8), 8)
        slot = _divmod2(b, _RING)[1]
        return _Block(wq_hbm.at[:, :, r], wq_buf.at[:, :, r], ring.at[slot], 1,
                      (wo_hbm.at[:, r], wo_buf.at[:, r], ring2.at[slot]))

    def mlp_blk(b):
        if b < n3:
            r = pl.ds(b * 8, 8)
            return _Block(w3_hbm.at[:, r], w3_buf.at[:, r], ring.at[b % _RING], 1)
        if b < n3 + n4:
            r = pl.ds((b - n3) * _R4, _R4)
            return _Block(w4_hbm.at[:, r], w4_buf.at[:, r], ring.at[b % _RING], 1)
        return None

    def kv_stream(src, buf, i):
        def blk(j):
            row, col = j // (nkv // 2) * dh, j % (nkv // 2) * 128
            return _Block(src.at[pl.ds(_mul(i, pr, 8) + row, dh), pl.ds(start + col, 128)],
                          buf.at[i % 2, pl.ds(row, dh), pl.ds(col, 128)],
                          ring.at[j % _RING], _KV_HI)
        return blk

    k_of = functools.partial(kv_stream, kt_hbm, k_buf)
    v_of = functools.partial(kv_stream, vt_hbm, v_buf)

    x_cp = pltpu.make_async_copy(x_hbm, x_buf, x_sem.at[0])
    x_cp.start()
    for b in range(_PRO_LO):
        w_blk(b).lo()

    def first(b, c):
        w_blk(b).hi()
        w_blk(b + _PRO_LO).lo()
        return c
    lax.fori_loop(0, _LOOK_HI, first, 0)
    for b in range(_PRO_LO + _LOOK_HI, _LOOK_LO):
        w_blk(b).lo()

    def w_tick(b, c):
        w_blk(b).wait()
        w_blk(b + _LOOK_HI).hi()
        w_blk(b + _LOOK_LO).lo()
        return c
    lax.fori_loop(0, _GT - _LOOK_LO, w_tick, 0)
    x_cp.wait()
    x = jnp.broadcast_to(x_buf[0].astype(_F32), (_ROWS, d))
    xn = _layernorm(x).astype(_BF16)
    for j in range(_GT - _LOOK_LO, _GT):
        _tick(j, _GT, w_blk, k_of(0))

    n_pv = 2 * _CHUNKS + 2
    n_q = pr // 128

    def q_slice(t, i):
        tpr = n_heads * dh // 128
        span = wq_buf.shape[1] * _GT // tpr
        parts = []
        for r in range(span):
            g, tile = _divmod2(r * tpr + i * n_q + t, _GT)
            parts.append(wq_buf[:, g, pl.ds(_mul(tile, 8, 8), 8), :])
        w = jnp.concatenate(parts, axis=1).reshape(d, 128)
        q_scr[:, t * 128:(t + 1) * 128] = jnp.dot(
            xn, w, preferred_element_type=_F32).astype(_BF16)

    def wo_rows(h):
        tpr = d // 128
        n = dh * tpr // 64
        parts = []
        for k in range(n):
            g, run = _divmod2(h * n + k, _GT // 8)
            parts.append(wo_buf[g, pl.ds(_mul(run, 64, 64), 64), :])
        t = jnp.concatenate(parts, axis=0).reshape(dh // 16, 16 * tpr, 128)
        cols = [jnp.concatenate([t[:, 8 * c:8 * c + 8], t[:, 8 * (tpr + c):8 * (tpr + c) + 8]],
                                axis=1).reshape(dh, 128) for c in range(tpr)]
        return jnp.concatenate(cols, axis=1)

    def pv_slice(j, i, l, o, attn):
        if j < 2 * _CHUNKS:
            hh, c = divmod(j, _CHUNKS)
            cols = slice(c * cw, (c + 1) * cw)
            oj = lax.dot_general(p_scr[hh, :, cols], v_buf[i % 2, hh * dh:(hh + 1) * dh, cols],
                                 _NT, preferred_element_type=_F32)
            o[hh] = oj if o[hh] is None else oj + o[hh]
        else:
            hh = j - 2 * _CHUNKS
            attn = attn + jnp.dot((o[hh] / l[hh]).astype(_BF16), wo_rows(2 * i + hh),
                                  preferred_element_type=_F32)
        return attn

    def k_phase(i, l, attn):
        o = [None, None]
        for j in range(nkv):
            _tick(j, nkv, k_of(i), v_of(i))
            if j % _STRIDE:
                continue
            jj = j // _STRIDE
            if jj < n_pv and l is not None:
                attn = pv_slice(jj, i - 1, l, o, attn)
            elif n_pv <= jj < n_pv + n_q:
                q_slice(jj - n_pv, i)
        return attn

    def v_phase(i, nxt, stride=_STRIDE, after=None):
        m = [None, None]
        l = [None, None]
        qh = None
        for j in range(nkv):
            _tick(j, nkv, v_of(i), nxt)
            if j % stride:
                continue
            jj = j // stride
            if jj == 0:
                qq = q_scr[...]
                qh = [qq[:, :dh], qq[:, dh:]]
            if jj < 2 * _CHUNKS:
                hh, c = divmod(jj, _CHUNKS)
                cols = slice(c * cw, (c + 1) * cw)
                s = jnp.dot(qh[hh], k_buf[i % 2, hh * dh:(hh + 1) * dh, cols],
                            preferred_element_type=_F32) * scale
                s_scr[hh, :, cols] = s
                for c2 in range(cw // 128):
                    sc = s[:, c2 * 128:(c2 + 1) * 128]
                    m[hh] = sc if m[hh] is None else jnp.maximum(m[hh], sc)
            elif jj == 2 * _CHUNKS:
                m = [jnp.max(mm, axis=-1, keepdims=True) for mm in m]
            elif jj <= 2 * _CHUNKS + 2:
                hh = jj - (2 * _CHUNKS + 1)
                p = jnp.exp(s_scr[hh] - m[hh])
                p_scr[hh] = p.astype(_BF16)
                l[hh] = jnp.sum(p, axis=-1, keepdims=True)
            elif after is not None:
                after(j)
        return l

    def pair(i, attn):
        l = v_phase(i, k_of(i + 1))
        return k_phase(i + 1, l, attn)

    assert (n_pv + n_q - 1) * _STRIDE < nkv
    k_phase(0, None, None)
    last = n_pairs - 1
    attn = lax.fori_loop(0, last, pair, jnp.zeros(x.shape, _F32))

    o = [None, None]
    todo = list(range(n_pv))

    def early_pv(j):
        if todo[0] < 2 * _CHUNKS and j + 1 >= (cw // 128) * (todo[0] + 1):
            pv_slice(todo.pop(0), last, None, o, None)

    l = v_phase(last, mlp_blk, 2, early_pv)

    no_more = lambda b: None
    out = y = z = None
    for j in range(n3):
        _tick(j, n3 + n4, mlp_blk, no_more)
        if todo:
            attn = pv_slice(todo.pop(0), last, l, o, attn)
        elif out is None:
            hres = x + attn
            y = _layernorm(hres)
            out = hres + y
        elif z is None:
            z = _layernorm(y).astype(_BF16)

    rg = w4_buf.shape[1]
    offs = [sum(_W4_STEPS[:k]) * _R4 for k in range(len(_W4_STEPS) + 1)]
    fs = f // _W3_SLICES
    n_mxu = len(_W4_STEPS) - _VPU_STEPS
    acts, gs, gcol = [], None, None
    b = n3
    for step, n in enumerate(_W4_STEPS):
        for t in range(n):
            if step == 0 and t < _W3_SLICES:
                w = w3_buf[:, :, t * fs:(t + 1) * fs].reshape(d, fs)
                a = jnp.dot(z, w, preferred_element_type=_F32)
                acts.append(jax.nn.gelu(a, approximate=True).astype(_BF16))
            elif step == 0 and t == _W3_SLICES:
                g = jnp.concatenate(acts, axis=1)
                gs = [jnp.concatenate([g[:, k * rg + r0:k * rg + r1] for k in range(_G4)], axis=1)
                      for r0, r1 in zip(offs[:-1], offs[1:])]
                gl = jnp.concatenate(gs[n_mxu:], axis=1)
                nl = gl.shape[1]
                eye = (lax.broadcasted_iota(jnp.int32, (nl, nl), 0)
                       == lax.broadcasted_iota(jnp.int32, (nl, nl), 1))
                diag = jnp.where(eye, jnp.broadcast_to(gl[0:1].astype(_F32), (nl, nl)), 0.0)
                gcol = jnp.dot(diag.astype(_BF16), jnp.ones((nl, 128), _BF16),
                               preferred_element_type=_F32)
            _tick(b, n3 + n4, mlp_blk, no_more)
            b += 1
        r0, r1 = offs[step], offs[step + 1]
        w = w4_buf[:, r0:r1, :].reshape(_G4 * (r1 - r0), d)
        if step < n_mxu:
            out = out + jnp.dot(gs[step], w, preferred_element_type=_F32)
            if step == n_mxu - 1:
                out = jnp.where(lax.broadcasted_iota(jnp.int32, out.shape, 0) == 0, out, 0.0)
        else:
            g0 = _G4 * (r0 - offs[n_mxu])
            gc = gcol[g0:g0 + w.shape[0]]
            prod = w.astype(_F32) * jnp.concatenate([gc] * (d // 128), axis=1)
            out = out + jnp.sum(prod.reshape(w.shape[0] // _ROWS, _ROWS, d), axis=0)
    out = jnp.sum(out, axis=0, keepdims=True)
    o_ref[0] = out.astype(o_ref.dtype)


def _kernel(*refs, **static):
    dma = pltpu.SemaphoreType.DMA
    pl.run_scoped(functools.partial(_body, *refs, **static),
                  dma((1,)), dma((_RING,)), dma((_RING,)))


@jax.jit
def pallas_sequential_preLN__sliding_block_cached__mixer_s_mlp__decode_kernel(
    A_x: jax.Array,
    A_k_cache: jax.Array,
    A_v_cache: jax.Array,
    A_wq: jax.Array,
    A_wo: jax.Array,
    B_x: jax.Array,
    B_w1: jax.Array,
    B_w2: jax.Array,
    B_w3: jax.Array,
    B_w4: jax.Array,
):
    b, sq, d = A_x.shape
    _, n_heads, sk, dh = A_k_cache.shape
    win = min(4096, max(256, sk // 4))
    f = B_w3.shape[1]
    assert (b, sq, d, n_heads, dh, win, f) == (1, 1, 640, 32, 192, 4096, 1536)
    assert f == _G4 * _R4 * sum(_W4_STEPS)

    kt = jnp.swapaxes(A_k_cache, 2, 3).reshape(n_heads * dh, sk)
    vt = jnp.swapaxes(A_v_cache, 2, 3).reshape(n_heads * dh, sk)
    tiles = lambda w: w.reshape(w.shape[0] // 8, 8, w.shape[1] // 128, 128).transpose(0, 2, 1, 3)
    wq = tiles(A_wq).reshape(d // 128, -1, _GT * 8, 128)
    wo = tiles(A_wo).reshape(-1, _GT * 8, 128)
    grouped = lambda w, g: w.reshape(g, w.shape[0] // g, w.shape[1])
    w3, w4 = grouped(B_w3, _G3), grouped(B_w4, _G4)

    any_spec = pl.BlockSpec(memory_space=pl.ANY)
    return pl.pallas_call(
        functools.partial(_kernel, n_heads=n_heads, dh=dh, sk=sk, win=win),
        in_specs=[any_spec] * 7,
        out_specs=pl.BlockSpec(memory_space=pltpu.VMEM),
        out_shape=jax.ShapeDtypeStruct(A_x.shape, A_x.dtype),
        scratch_shapes=[
            pltpu.VMEM(A_x.shape, _BF16),
            pltpu.VMEM(wq.shape, _BF16),
            pltpu.VMEM(wo.shape, _BF16),
            pltpu.VMEM(w3.shape, _BF16),
            pltpu.VMEM(w4.shape, _BF16),
            pltpu.VMEM((2, 2 * dh, win), _BF16),
            pltpu.VMEM((2, 2 * dh, win), _BF16),
            pltpu.VMEM((_ROWS, 2 * dh), _BF16),
            pltpu.VMEM((2, _ROWS, win), _F32),
            pltpu.VMEM((2, _ROWS, win), _BF16),
        ],
        compiler_params=pltpu.CompilerParams(vmem_limit_bytes=64 * 1024 * 1024),
    )(A_x, kt, vt, wq, wo, w3, w4)
```

```python
import functools

import jax
import jax.numpy as jnp
from jax import lax
import jax.experimental.pallas as pl
import jax.experimental.pallas.tpu as pltpu

_F32 = jnp.float32
_BF16 = jnp.bfloat16
_EPS = 1e-5
_ROWS = 8
_NT = (((1,), (1,)), ((), ()))

_LOOK_HI = 15
_LOOK_LO = 28
_PRO_LO = 2
_RING = 64
_KV_HI = 32
_STRIDE = 3
_CHUNKS = 8
_GT = 256
_G3, _G4, _R4 = 4, 4, 16
_W3_SLICES = 6
_W4_STEPS = (8, 8, 5, 1, 1, 1)
_VPU_STEPS = 3


def _layernorm(x):
    m = jnp.mean(x, axis=-1, keepdims=True)
    xc = x - m
    v = jnp.mean(xc * xc, axis=-1, keepdims=True)
    return xc / jnp.sqrt(v + _EPS)


def _mul(i, n, align):
    return i * n if isinstance(i, int) else pl.multiple_of(i * n, align)


def _divmod2(i, n):
    if isinstance(i, int):
        return divmod(i, n)
    return lax.shift_right_logical(i, n.bit_length() - 1), lax.bitwise_and(i, n - 1)


class _Block:
    def __init__(self, src, dst, sem, n_hi, extra=None):
        self.src, self.dst, self.sem, self.n_hi, self.extra = src, dst, sem, n_hi, extra

    def _piece(self, a, n):
        return pltpu.make_async_copy(
            self.src.at[pl.ds(a, n)], self.dst.at[pl.ds(a, n)], self.sem)

    def hi(self):
        self._piece(0, self.n_hi).start(priority=0)

    def lo(self):
        self._piece(self.n_hi, self.dst.shape[0] - self.n_hi).start(priority=1)
        if self.extra is not None:
            pltpu.make_async_copy(*self.extra).start(priority=1)

    def wait(self):
        pltpu.make_async_copy(self.dst, self.dst, self.sem).wait()
        if self.extra is not None:
            pltpu.make_async_copy(*self.extra).wait()


def _tick(j, n, cur, nxt):
    cur(j).wait()
    ahead = lambda p: cur(p) if p < n else nxt(p - n)
    bh, bl = ahead(j + _LOOK_HI), ahead(j + _LOOK_LO)
    if bh is not None:
        bh.hi()
    if bl is not None:
        bl.lo()


def _body(x_hbm, kt_hbm, vt_hbm, wq_hbm, wo_hbm, w3_hbm, w4_hbm, o_ref,
          x_buf, wq_buf, wo_buf, w3_buf, w4_buf, k_buf, v_buf, q_scr, s_scr, p_scr,
          x_sem, ring, ring2, *, n_heads, dh, sk, win):
    start = sk - win
    scale = dh ** -0.5
    d = x_buf.shape[-1]
    f = w3_buf.shape[-1]
    pr = 2 * dh
    n_pairs = n_heads // 2
    n3 = w3_buf.shape[1] // 8
    n4 = w4_buf.shape[1] // _R4
    nkv = 2 * (win // 128)
    assert nkv % _RING == 0 and _GT % _RING == 0 and _LOOK_LO < _RING

    def w_blk(b):
        r = pl.ds(_mul(b, 8, 8), 8)
        slot = _divmod2(b, _RING)[1]
        return _Block(wq_hbm.at[:, :, r], wq_buf.at[:, :, r], ring.at[slot], 1,
                      (wo_hbm.at[:, r], wo_buf.at[:, r], ring2.at[slot]))

    def mlp_blk(b):
        if b < n3:
            r = pl.ds(b * 8, 8)
            return _Block(w3_hbm.at[:, r], w3_buf.at[:, r], ring.at[b % _RING], 1)
        if b < n3 + n4:
            r = pl.ds((b - n3) * _R4, _R4)
            return _Block(w4_hbm.at[:, r], w4_buf.at[:, r], ring.at[b % _RING], 1)
        return None

    def kv_stream(src, buf, i):
        def blk(j):
            row, col = j // (nkv // 2) * dh, j % (nkv // 2) * 128
            return _Block(src.at[pl.ds(_mul(i, pr, 8) + row, dh), pl.ds(start + col, 128)],
                          buf.at[i % 2, pl.ds(row, dh), pl.ds(col, 128)],
                          ring.at[j % _RING], _KV_HI)
        return blk

    k_of = functools.partial(kv_stream, kt_hbm, k_buf)
    v_of = functools.partial(kv_stream, vt_hbm, v_buf)

    x_cp = pltpu.make_async_copy(x_hbm, x_buf, x_sem.at[0])
    x_cp.start()
    for b in range(_PRO_LO):
        w_blk(b).lo()

    def first(b, c):
        w_blk(b).hi()
        w_blk(b + _PRO_LO).lo()
        return c
    lax.fori_loop(0, _LOOK_HI, first, 0)
    for b in range(_PRO_LO + _LOOK_HI, _LOOK_LO):
        w_blk(b).lo()

    def w_tick(b, c):
        w_blk(b).wait()
        w_blk(b + _LOOK_HI).hi()
        w_blk(b + _LOOK_LO).lo()
        return c
    lax.fori_loop(0, _GT - _LOOK_LO, w_tick, 0)
    x_cp.wait()
    x = jnp.broadcast_to(x_buf[0].astype(_F32), (_ROWS, d))
    xn = _layernorm(x).astype(_BF16)
    for j in range(_GT - _LOOK_LO, _GT):
        _tick(j, _GT, w_blk, k_of(0))

    n_pv = 2 * _CHUNKS + 2
    n_q = pr // 128

    def q_slice(t, i):
        tpr = n_heads * dh // 128
        span = wq_buf.shape[1] * _GT // tpr
        parts = []
        for r in range(span):
            g, tile = _divmod2(r * tpr + i * n_q + t, _GT)
            parts.append(wq_buf[:, g, pl.ds(_mul(tile, 8, 8), 8), :])
        w = jnp.concatenate(parts, axis=1).reshape(d, 128)
        q_scr[:, t * 128:(t + 1) * 128] = jnp.dot(
            xn, w, preferred_element_type=_F32).astype(_BF16)

    def wo_rows(h):
        tpr = d // 128
        n = dh * tpr // 64
        parts = []
        for k in range(n):
            g, run = _divmod2(h * n + k, _GT // 8)
            parts.append(wo_buf[g, pl.ds(_mul(run, 64, 64), 64), :])
        t = jnp.concatenate(parts, axis=0).reshape(dh // 16, 16 * tpr, 128)
        cols = [jnp.concatenate([t[:, 8 * c:8 * c + 8], t[:, 8 * (tpr + c):8 * (tpr + c) + 8]],
                                axis=1).reshape(dh, 128) for c in range(tpr)]
        return jnp.concatenate(cols, axis=1)

    def pv_slice(j, i, l, o, attn, nch=_CHUNKS):
        cw = win // nch
        if j < 2 * nch:
            hh, c = divmod(j, nch)
            cols = slice(c * cw, (c + 1) * cw)
            oj = lax.dot_general(p_scr[hh, :, cols], v_buf[i % 2, hh * dh:(hh + 1) * dh, cols],
                                 _NT, preferred_element_type=_F32)
            o[hh] = oj if o[hh] is None else oj + o[hh]
        else:
            hh = j - 2 * nch
            attn = attn + jnp.dot((o[hh] / l[hh]).astype(_BF16), wo_rows(2 * i + hh),
                                  preferred_element_type=_F32)
        return attn

    def k_phase(i, l, attn):
        o = [None, None]
        for j in range(nkv):
            _tick(j, nkv, k_of(i), v_of(i))
            if j % _STRIDE:
                continue
            jj = j // _STRIDE
            if jj < n_pv and l is not None:
                attn = pv_slice(jj, i - 1, l, o, attn)
            elif n_pv <= jj < n_pv + n_q:
                q_slice(jj - n_pv, i)
        return attn

    def v_phase(i, nxt, nch=_CHUNKS, after=None):
        cw = win // nch
        m = [None, None]
        l = [None, None]
        qh = None
        for j in range(nkv):
            _tick(j, nkv, v_of(i), nxt)
            if j % _STRIDE:
                continue
            jj = j // _STRIDE
            if jj == 0:
                qq = q_scr[...]
                qh = [qq[:, :dh], qq[:, dh:]]
            if jj < 2 * nch:
                hh, c = divmod(jj, nch)
                cols = slice(c * cw, (c + 1) * cw)
                s = jnp.dot(qh[hh], k_buf[i % 2, hh * dh:(hh + 1) * dh, cols],
                            preferred_element_type=_F32) * scale
                s_scr[hh, :, cols] = s
                for c2 in range(cw // 128):
                    sc = s[:, c2 * 128:(c2 + 1) * 128]
                    m[hh] = sc if m[hh] is None else jnp.maximum(m[hh], sc)
            elif jj == 2 * nch:
                m = [jnp.max(mm, axis=-1, keepdims=True) for mm in m]
            elif jj <= 2 * nch + 2:
                hh = jj - (2 * nch + 1)
                p = jnp.exp(s_scr[hh] - m[hh])
                p_scr[hh] = p.astype(_BF16)
                l[hh] = jnp.sum(p, axis=-1, keepdims=True)
            elif after is not None:
                after(j)
        return l

    def pair(i, attn):
        l = v_phase(i, k_of(i + 1))
        return k_phase(i + 1, l, attn)

    assert (n_pv + n_q - 1) * _STRIDE < nkv
    k_phase(0, None, None)
    last = n_pairs - 1
    attn = lax.fori_loop(0, last, pair, jnp.zeros(x.shape, _F32))

    o = [None, None]
    nch = _CHUNKS // 2
    todo = list(range(2 * nch + 2))

    def early_pv(j):
        if todo[0] < 2 * nch and j + 1 >= nkv // (2 * nch) * (todo[0] + 1):
            pv_slice(todo.pop(0), last, None, o, None, nch)

    l = v_phase(last, mlp_blk, nch, early_pv)

    no_more = lambda b: None
    out = y = z = None
    for j in range(n3):
        _tick(j, n3 + n4, mlp_blk, no_more)
        if todo:
            attn = pv_slice(todo.pop(0), last, l, o, attn, nch)
        elif out is None:
            hres = x + attn
            y = _layernorm(hres)
            out = hres + y
        elif z is None:
            z = _layernorm(y).astype(_BF16)

    rg = w4_buf.shape[1]
    offs = [sum(_W4_STEPS[:k]) * _R4 for k in range(len(_W4_STEPS) + 1)]
    fs = f // _W3_SLICES
    n_mxu = len(_W4_STEPS) - _VPU_STEPS
    acts, gs, gcol = [], None, None
    b = n3
    for step, n in enumerate(_W4_STEPS):
        for t in range(n):
            if step == 0 and t < _W3_SLICES:
                w = w3_buf[:, :, t * fs:(t + 1) * fs].reshape(d, fs)
                a = jnp.dot(z, w, preferred_element_type=_F32)
                acts.append(jax.nn.gelu(a, approximate=True).astype(_BF16))
            elif step == 0 and t == _W3_SLICES:
                g = jnp.concatenate(acts, axis=1)
                gs = [jnp.concatenate([g[:, k * rg + r0:k * rg + r1] for k in range(_G4)], axis=1)
                      for r0, r1 in zip(offs[:-1], offs[1:])]
                gl = jnp.concatenate(gs[n_mxu:], axis=1)
                nl = gl.shape[1]
                eye = (lax.broadcasted_iota(jnp.int32, (nl, nl), 0)
                       == lax.broadcasted_iota(jnp.int32, (nl, nl), 1))
                diag = jnp.where(eye, jnp.broadcast_to(gl[0:1].astype(_F32), (nl, nl)), 0.0)
                gcol = jnp.dot(diag.astype(_BF16), jnp.ones((nl, 128), _BF16),
                               preferred_element_type=_F32)
            _tick(b, n3 + n4, mlp_blk, no_more)
            b += 1
        r0, r1 = offs[step], offs[step + 1]
        w = w4_buf[:, r0:r1, :].reshape(_G4 * (r1 - r0), d)
        if step < n_mxu:
            out = out + jnp.dot(gs[step], w, preferred_element_type=_F32)
            if step == n_mxu - 1:
                out = jnp.where(lax.broadcasted_iota(jnp.int32, out.shape, 0) == 0, out, 0.0)
        else:
            g0 = _G4 * (r0 - offs[n_mxu])
            gc = gcol[g0:g0 + w.shape[0]]
            prod = w.astype(_F32) * jnp.concatenate([gc] * (d // 128), axis=1)
            out = out + jnp.sum(prod.reshape(w.shape[0] // _ROWS, _ROWS, d), axis=0)
    out = jnp.sum(out, axis=0, keepdims=True)
    o_ref[0] = out.astype(o_ref.dtype)


def _kernel(*refs, **static):
    dma = pltpu.SemaphoreType.DMA
    pl.run_scoped(functools.partial(_body, *refs, **static),
                  dma((1,)), dma((_RING,)), dma((_RING,)))


@jax.jit
def pallas_sequential_preLN__sliding_block_cached__mixer_s_mlp__decode_kernel(
    A_x: jax.Array,
    A_k_cache: jax.Array,
    A_v_cache: jax.Array,
    A_wq: jax.Array,
    A_wo: jax.Array,
    B_x: jax.Array,
    B_w1: jax.Array,
    B_w2: jax.Array,
    B_w3: jax.Array,
    B_w4: jax.Array,
):
    b, sq, d = A_x.shape
    _, n_heads, sk, dh = A_k_cache.shape
    win = min(4096, max(256, sk // 4))
    f = B_w3.shape[1]
    assert (b, sq, d, n_heads, dh, win, f) == (1, 1, 640, 32, 192, 4096, 1536)
    assert f == _G4 * _R4 * sum(_W4_STEPS)

    kt = jnp.swapaxes(A_k_cache, 2, 3).reshape(n_heads * dh, sk)
    vt = jnp.swapaxes(A_v_cache, 2, 3).reshape(n_heads * dh, sk)
    tiles = lambda w: w.reshape(w.shape[0] // 8, 8, w.shape[1] // 128, 128).transpose(0, 2, 1, 3)
    wq = tiles(A_wq).reshape(d // 128, -1, _GT * 8, 128)
    wo = tiles(A_wo).reshape(-1, _GT * 8, 128)
    grouped = lambda w, g: w.reshape(g, w.shape[0] // g, w.shape[1])
    w3, w4 = grouped(B_w3, _G3), grouped(B_w4, _G4)

    any_spec = pl.BlockSpec(memory_space=pl.ANY)
    return pl.pallas_call(
        functools.partial(_kernel, n_heads=n_heads, dh=dh, sk=sk, win=win),
        in_specs=[any_spec] * 7,
        out_specs=pl.BlockSpec(memory_space=pltpu.VMEM),
        out_shape=jax.ShapeDtypeStruct(A_x.shape, A_x.dtype),
        scratch_shapes=[
            pltpu.VMEM(A_x.shape, _BF16),
            pltpu.VMEM(wq.shape, _BF16),
            pltpu.VMEM(wo.shape, _BF16),
            pltpu.VMEM(w3.shape, _BF16),
            pltpu.VMEM(w4.shape, _BF16),
            pltpu.VMEM((2, 2 * dh, win), _BF16),
            pltpu.VMEM((2, 2 * dh, win), _BF16),
            pltpu.VMEM((_ROWS, 2 * dh), _BF16),
            pltpu.VMEM((2, _ROWS, win), _F32),
            pltpu.VMEM((2, _ROWS, win), _BF16),
        ],
        compiler_params=pltpu.CompilerParams(vmem_limit_bytes=64 * 1024 * 1024),
    )(A_x, kt, vt, wq, wo, w3, w4)
```
